```python
import jax
import jax.numpy as jnp

def _softmax(x, axis=-1):
    return jax.nn.softmax(x, axis=axis)

def _gelu(x):
    return jax.nn.gelu(x, approximate=True)

def _silu(x):
    return jax.nn.silu(x)

def _sigmoid(x):
    return jax.nn.sigmoid(x)

def _layernorm(x, axis=-1, eps=1e-05):
    m = jnp.mean(x, axis=axis, keepdims=True)
    v = jnp.var(x, axis=axis, keepdims=True)
    return (x - m) / jnp.sqrt(v + eps)

def _scatter_add(tgt, idx, src, axis=0):
    return tgt.at[idx].add(src)

def _segment_sum(src, seg, n):
    return jax.ops.segment_sum(src, seg, n)

class _Rng:

    def __init__(self, key):
        self._k = key

    def _next(self):
        self._k, sub = jax.random.split(self._k)
        return sub

    def normal(self, shape):
        return jax.random.normal(self._next(), shape, dtype=jnp.bfloat16)

    def randint(self, lo, hi, shape):
        return jax.random.randint(self._next(), shape, lo, hi, dtype=jnp.int32)

    def uniform(self, shape, lo=0.0, hi=1.0):
        return jax.random.uniform(self._next(), shape, jnp.bfloat16, lo, hi)

    def permutation(self, n):
        return jax.random.permutation(self._next(), n)
kernel_name = 'interleave_layers__memory_aug_recurrent_mem_tr__sliding_local_dilated__prompt'

def setup_inputs():
    _rng = _Rng(jax.random.key(int.from_bytes(__import__("os").urandom(4), "little")))
    _w = lambda a: (lambda t: t.astype(jnp.bfloat16) if jnp.issubdtype(t.dtype, jnp.floating) else t)(jnp.asarray(a))

    def _A_setup():
        B, S, Dm = (1, 2048, 640)
        H, Dh = (32, 192)
        M, seg = (8, 32)
        seg = min(seg, S)
        S = S // seg * seg
        return {'x': _w((lambda *s: _rng.normal(s) * 0.05)(B, S, Dm)), 'mem0': _w((lambda *s: _rng.normal(s) * 0.05)(B, M, Dm)), 'Wq': _w((lambda *s: _rng.normal(s) * 0.05)(Dm, H, Dh) * Dm ** (-0.5)), 'Wk': _w((lambda *s: _rng.normal(s) * 0.05)(Dm, H, Dh) * Dm ** (-0.5)), 'Wv': _w((lambda *s: _rng.normal(s) * 0.05)(Dm, H, Dh) * Dm ** (-0.5)), 'Wo': _w((lambda *s: _rng.normal(s) * 0.05)(H, Dh, Dm) * (H * Dh) ** (-0.5)), 'seg_len': seg}
    _A_in = _A_setup()

    def _B_setup():
        B, S, D = (1, 2048, 640)
        return {'x': _w((lambda *s: _rng.normal(s) * 0.05)(B, S, D)), 'wqkv': _w((lambda *s: _rng.normal(s) * 0.05)(D, 3 * D)), 'wo': _w((lambda *s: _rng.normal(s) * 0.05)(D, D))}
    _B_in = _B_setup()
    return {'A_x': _A_in['x'], 'A_mem0': _A_in['mem0'], 'A_Wq': _A_in['Wq'], 'A_Wk': _A_in['Wk'], 'A_Wv': _A_in['Wv'], 'A_Wo': _A_in['Wo'], 'A_seg_len': _A_in['seg_len'], 'B_x': _B_in['x'], 'B_wqkv': _B_in['wqkv'], 'B_wo': _B_in['wo']}

def reference(A_x, A_mem0, A_Wq, A_Wk, A_Wv, A_Wo, A_seg_len, B_x, B_wqkv, B_wo):

    def _A_ref(x, mem0, Wq, Wk, Wv, Wo, seg_len):
        B, S, Dm = x.shape
        H, Dh = (Wq.shape[1], Wq.shape[2])
        M = mem0.shape[1]
        scale = Dh ** (-0.5)
        n_seg = S // seg_len
        L = M + seg_len
        idx = jnp.arange(L)
        mask = (idx[:, None] < M) | (idx[:, None] >= idx[None, :])
        mem = mem0
        outs = []
        for s in range(n_seg):
            xs = x[:, s * seg_len:(s + 1) * seg_len, :].copy()
            h = jnp.concatenate([mem, xs], axis=1)
            q = jnp.einsum('btd,dhe->bhte', h, Wq)
            k = jnp.einsum('btd,dhe->bhte', h, Wk)
            v = jnp.einsum('btd,dhe->bhte', h, Wv)
            scores = jnp.einsum('bhqe,bhke->bhqk', q, k) * scale
            scores = jnp.where(mask[None, None], scores, -1000000000.0)
            p = _softmax(scores, axis=-1)
            o = jnp.einsum('bhqk,bhke->bhqe', p, v)
            o = jnp.einsum('bhte,hed->btd', o, Wo)
            mem = o[:, :M, :].copy()
            outs.append(o[:, M:, :])
        return jnp.concatenate(outs, axis=1)

    def _B_ref(x, wqkv, wo):
        B, S, D = x.shape
        H = 32
        Dh = D // H
        W, dil = (8, 2)
        qkv = (lambda x, *d: x.transpose(*d))((x @ wqkv).reshape(B, S, 3, H, Dh), 2, 0, 3, 1, 4)
        q, k, v = (qkv[0], qkv[1], qkv[2])
        scale = Dh ** (-0.5)
        pos = jnp.arange(S)
        off = jnp.arange(W) * dil
        idx = pos[:, None] - off[None, :]
        mask = idx >= 0
        idx_c = jnp.where(mask, idx, 0).reshape(-1)
        kg = k[:, :, idx_c, :].reshape(B, H, S, W, Dh)
        vg = v[:, :, idx_c, :].reshape(B, H, S, W, Dh)
        logits = jnp.einsum('bhsd,bhswd->bhsw', q, kg) * scale
        logits = jnp.where(mask[None, None, :, :], logits, -1000000000.0)
        attn = _softmax(logits, axis=-1)
        o = jnp.einsum('bhsw,bhswd->bhsd', attn, vg)
        return (lambda x, *d: x.transpose(*d))(o, 0, 2, 1, 3).reshape(B, S, D) @ wo
    x = A_x
    x = x + _A_ref(_layernorm(x, axis=-1), A_mem0, A_Wq, A_Wk, A_Wv, A_Wo, A_seg_len)
    x = x + _B_ref(_layernorm(x, axis=-1), B_wqkv, B_wo)
    x = x + _A_ref(_layernorm(x, axis=-1), A_mem0, A_Wq, A_Wk, A_Wv, A_Wo, A_seg_len)
    x = x + _B_ref(_layernorm(x, axis=-1), B_wqkv, B_wo)
    return x
```

```python
import functools

import jax
import jax.numpy as jnp
import numpy as np
from jax import lax
from jax.experimental import pallas as pl
from jax.experimental.pallas import tpu as pltpu

F32 = jnp.float32
BF16 = jnp.bfloat16
U32 = jnp.uint32
NEG = -1000000000.0
OUT_LAG = 3
UNROLL = 1


def _bf16_const(v):
    return float(np.asarray(v, dtype=BF16).astype(np.float32))


def _dot(a, b):
    return lax.dot_general(a, b, (((1,), (0,)), ((), ())), preferred_element_type=F32)


def _dot_nt(a, b):
    return lax.dot_general(a, b, (((1,), (1,)), ((), ())), preferred_element_type=F32)


def _layernorm(x):
    m = jnp.mean(x, axis=-1, keepdims=True)
    c = x - m
    v = jnp.mean(c * c, axis=-1, keepdims=True)
    return c * lax.rsqrt(v + 1e-5)


def _w(ref_slice):
    return pltpu.bitcast(ref_slice, BF16)


def _recip(d):
    r = pl.reciprocal(d, approx=True)
    return r * (2.0 - d * r)


def _kernel(x_ref, mem0_ref, wq_ref, wk_ref, wv_ref, wo_ref, bqkv_ref, bwo_ref,
            out_ref,
            xs, w_s, wo_s, bqkv_s, bwo_s, hbuf, hbbuf, qbuf, kbuf, vbuf,
            *, S, D, H, DH, M, SEG, W, DIL, HB):
    NSEG = S // SEG
    NG = 2 * NSEG
    L = M + SEG
    NP = H // 2
    PW = 2 * DH
    a_scale = _bf16_const(DH ** -0.5)
    b_scale = _bf16_const((D // HB) ** -0.5)
    TAIL = 16
    NT = D // 128

    for p in range(NP):
        c = slice(p * PW, (p + 1) * PW)
        for j, ref in enumerate((wq_ref, wk_ref, wv_ref)):
            w_s[:, (3 * p + j) * PW:(3 * p + j + 1) * PW] = pltpu.bitcast(ref[:, c], U32)
        wo_s[p * DH:(p + 1) * DH, :] = pltpu.bitcast(wo_ref[c, :], U32)
    for j in range(3):
        c = slice(j * D, (j + 1) * D)
        bqkv_s[:, c] = pltpu.bitcast(bqkv_ref[:, c], U32)
    bwo_s[...] = pltpu.bitcast(bwo_ref[...], U32)
    for i in range(S // 256):
        xs[i * 256:(i + 1) * 256, :] = x_ref[i * 256:(i + 1) * 256, :].astype(F32)
    kbuf[...] = jnp.zeros(kbuf.shape, F32)
    vbuf[...] = jnp.zeros(vbuf.shape, F32)
    qbuf[...] = jnp.zeros(qbuf.shape, F32)
    hbbuf[...] = jnp.zeros(hbbuf.shape, F32)
    mem0 = mem0_ref[...].astype(F32)
    hbuf[...] = _layernorm(xs[0:SEG, :])

    def rows(seg):
        return pl.ds(pl.multiple_of(seg * SEG, SEG), SEG)

    def b_ln(seg):
        hbbuf[...] = _layernorm(xs[rows(seg), :])

    def b_proj(seg, j):
        y = _dot(hbbuf[...], _w(bqkv_s[:, j * D:(j + 1) * D]))
        if j == 0:
            qbuf[...] = y * b_scale
        else:
            buf = kbuf if j == 1 else vbuf
            buf[0:TAIL, :] = jnp.where(seg == 0, 0.0, buf[SEG:SEG + TAIL, :])
            buf[TAIL:, :] = y

    def b_logit(st, seg, w):
        off = TAIL - DIL * w
        s = None
        for j in range(NT):
            c = slice(j * 128, (j + 1) * 128)
            t = qbuf[:, c] * kbuf[off:off + SEG, c]
            s = t if s is None else s + t
        s = s + pltpu.roll(s, 64, 1)
        s = s + pltpu.roll(s, 32, 1)
        if w > 0:
            pos = lax.broadcasted_iota(jnp.int32, (SEG, 128), 0) + seg * SEG
            s = jnp.where(pos >= DIL * w, s, NEG)
        st.setdefault("blog", []).append(s)

    def b_softmax(st):
        logits = st["blog"]
        m = functools.reduce(jnp.maximum, logits)
        es = [jnp.exp(s - m) for s in logits]
        st["bexp"] = es
        st["binv"] = _recip(functools.reduce(jnp.add, es))

    def b_pv(st, j):
        c = slice(j * 128, (j + 1) * 128)
        oj = None
        for w in range(W):
            off = TAIL - DIL * w
            t = st["bexp"][w] * vbuf[off:off + SEG, c]
            oj = t if oj is None else oj + t
        st.setdefault("bo", []).append(oj * st["binv"])

    def b_out(st, seg, active):
        o = jnp.concatenate(st["bo"], axis=1)
        x1 = xs[rows(seg), :]
        x2 = x1 + _dot(o, _w(bwo_s[...]))
        x2 = jnp.where(active, x2, x1)
        xs[rows(seg), :] = x2
        out_ref[rows(seg), :] = x2.astype(out_ref.dtype)

    def a_proj(st, p, j):
        c0 = (3 * p + j) * PW
        st["qkv"[j], p] = _dot(st["h"], _w(w_s[:, c0:c0 + PW]))

    def _split_heads(t):
        lane = lax.broadcasted_iota(jnp.int32, (L, 128), 1)
        lo = lane < (DH - 128)
        z = jnp.zeros((L, 128), F32)
        t0, t1, t2 = t[:, 0:128], t[:, 128:256], t[:, 256:384]
        top = jnp.concatenate([t0, jnp.where(lo, t1, 0.0), z], axis=1)
        bot = jnp.concatenate([z, jnp.where(lo, 0.0, t1), t2], axis=1)
        return jnp.concatenate([top, bot], axis=0).astype(BF16)

    def a_qk(st, p):
        st["s", p] = _dot_nt(st["q", p], _split_heads(st["k", p]))

    def _smask():
        row = lax.broadcasted_iota(jnp.int32, (L, 2 * L), 0)
        col = lax.broadcasted_iota(jnp.int32, (L, 2 * L), 1)
        lo = col < L
        key = jnp.where(lo, col, col - L)
        return lo, (row < M) | (row >= key)

    def a_max(st, p):
        lo, mask = _smask()
        s = jnp.where(mask, st["s", p] * a_scale, NEG)
        m_lo = jnp.max(jnp.where(lo, s, -jnp.inf), axis=-1, keepdims=True)
        m_hi = jnp.max(jnp.where(lo, -jnp.inf, s), axis=-1, keepdims=True)
        st["s", p] = s
        st["m", p] = (m_lo, m_hi)

    def a_exp(st, p):
        lo, _ = _smask()
        m_lo, m_hi = st["m", p]
        e = jnp.exp(st["s", p] - jnp.where(lo, m_lo, m_hi))
        d_lo = jnp.sum(jnp.where(lo, e, 0.0), axis=-1, keepdims=True)
        d_hi = jnp.sum(jnp.where(lo, 0.0, e), axis=-1, keepdims=True)
        st["e", p] = e
        st["d", p] = (d_lo, d_hi)

    def a_pv(st, p):
        lo, _ = _smask()
        d_lo, d_hi = st["d", p]
        pr = st["e", p] * _recip(jnp.where(lo, d_lo, d_hi))
        st["o", p] = _dot(pr, _split_heads(st["v", p]))

    def a_out(st, p):
        y = _dot(st["o", p], _w(wo_s[p * DH:(p + 1) * DH, :]))
        st["acc"] = y if "acc" not in st else st["acc"] + y

    def step(g, mem):
        seg = g % NSEG
        seg1 = (g + NSEG - 1) % NSEG
        seg2 = (g + NSEG - 2) % NSEG
        segn = (g + 1) % NSEG
        mem = jnp.where(seg == 0, mem0, mem)
        st = {"h": jnp.concatenate([mem, hbuf[...]], axis=0)}

        bwork = [functools.partial(b_logit, st, seg2, w) for w in range(W)]
        bwork.append(functools.partial(b_softmax, st))
        bwork += [functools.partial(b_pv, st, j) for j in range(NT)]

        def bnext(n=1):
            for _ in range(n):
                if bwork:
                    bwork.pop(0)()

        a_proj(st, 0, 0)
        bnext()
        a_proj(st, 0, 1)
        bnext()
        a_proj(st, 0, 2)
        bnext()
        for p in range(NP + OUT_LAG):
            nxt = p + 1 < NP
            if nxt:
                a_proj(st, p + 1, 0)
            if p < NP:
                a_qk(st, p)
            if 1 <= p <= NP:
                a_pv(st, p - 1)
            if nxt:
                a_proj(st, p + 1, 1)
            if p < NP:
                a_max(st, p)
            if nxt:
                a_proj(st, p + 1, 2)
            if p < NP:
                a_exp(st, p)
            if p == NP - 1:
                bnext(100)
                b_ln(seg1)
            if p >= OUT_LAG:
                a_out(st, p - OUT_LAG)
            if p < NP - 1:
                bnext()
            if p == NP:
                b_out(st, seg2, g >= 2)
        bnext(100)
        acc = st["acc"]
        xs[rows(seg), :] = xs[rows(seg), :] + acc[M:, :]
        hbuf[...] = _layernorm(xs[rows(segn), :])
        for j in range(3):
            b_proj(seg1, j)
        return acc[:M, :]

    lax.fori_loop(0, NG, step, mem0, unroll=UNROLL)

    for i, seg in enumerate((NSEG - 2, NSEG - 1)):
        st = {}
        for w in range(W):
            b_logit(st, seg, w)
        b_softmax(st)
        for j in range(NT):
            b_pv(st, j)
        if i == 0:
            b_ln(NSEG - 1)
        b_out(st, seg, True)
        if i == 0:
            for j in range(3):
                b_proj(NSEG - 1, j)


@functools.partial(jax.jit, static_argnames=("A_seg_len",))
def pallas_interleave_layers__memory_aug_recurrent_mem_tr__sliding_local_dilated__prompt_kernel(A_x, A_mem0, A_Wq, A_Wk, A_Wv, A_Wo, A_seg_len, B_x, B_wqkv, B_wo):
    del B_x
    B, S, D = A_x.shape
    M = A_mem0.shape[1]
    _, H, DH = A_Wq.shape
    SEG = int(A_seg_len)
    HB, W, DIL = 32, 8, 2
    DB = D // HB
    x2 = A_x.reshape(S, D)
    mem0 = A_mem0.reshape(M, D)
    wq = A_Wq.reshape(D, H * DH)
    wk = A_Wk.reshape(D, H * DH)
    wv = A_Wv.reshape(D, H * DH)
    wo = A_Wo.reshape(H * DH, D)
    bqkv = B_wqkv.reshape(D, 3, HB, DB).transpose(0, 1, 3, 2).reshape(D, 3 * D)
    bwo = B_wo.reshape(HB, DB, D).transpose(1, 0, 2).reshape(D, D)
    out = pl.pallas_call(
        functools.partial(_kernel, S=S, D=D, H=H, DH=DH, M=M, SEG=SEG, W=W, DIL=DIL, HB=HB),
        out_shape=jax.ShapeDtypeStruct((S, D), A_x.dtype),
        scratch_shapes=[
            pltpu.VMEM((S, D), F32),
            pltpu.VMEM((D // 2, 3 * H * DH), U32),
            pltpu.VMEM((H * DH // 2, D), U32),
            pltpu.VMEM((D // 2, 3 * D), U32),
            pltpu.VMEM((D // 2, D), U32),
            pltpu.VMEM((SEG, D), F32),
            pltpu.VMEM((SEG, D), F32),
            pltpu.VMEM((SEG, D), F32),
            pltpu.VMEM((16 + SEG, D), F32),
            pltpu.VMEM((16 + SEG, D), F32),
        ],
        compiler_params=pltpu.CompilerParams(vmem_limit_bytes=120 * 1024 * 1024),
    )(x2, mem0, wq, wk, wv, wo, bqkv, bwo)
    return out.reshape(B, S, D)
```

```python
import functools

import jax
import jax.numpy as jnp
import numpy as np
from jax import lax
from jax.experimental import pallas as pl
from jax.experimental.pallas import tpu as pltpu

F32 = jnp.float32
BF16 = jnp.bfloat16
U32 = jnp.uint32
NEG = -1000000000.0

UNROLL = 3
AHEAD = 2


def _bf16_const(v):
    return float(np.asarray(v, dtype=BF16).astype(np.float32))


def _dot(a, b):
    return lax.dot_general(a, b, (((1,), (0,)), ((), ())), preferred_element_type=F32)


def _dot_nt(a, b):
    return lax.dot_general(a, b, (((1,), (1,)), ((), ())), preferred_element_type=F32)


def _layernorm(x):
    m = jnp.mean(x, axis=-1, keepdims=True)
    c = x - m
    v = jnp.mean(c * c, axis=-1, keepdims=True)
    return c * lax.rsqrt(v + 1e-5)


def _w(ref_slice):
    return pltpu.bitcast(ref_slice, BF16)


def _recip(d):
    r = pl.reciprocal(d, approx=True)
    return r * (2.0 - d * r)


LAG = 5
BOUT = 9
BLN = 12


def build_schedule(NP):
    s = [("q", 0), ("k", 0), ("v", 0)]
    bwork = [("blog", w) for w in range(8)] + [("bsm",)] + [("bpv", j) for j in range(5)]
    per = -(-len(bwork) // BOUT)
    nout = 0
    for p in range(NP):
        nxt = p + 1 < NP
        if not nxt:
            break
        s.append(("q", p + 1))
        s.append(("qk", p))
        if p >= 1:
            s.append(("pv", p - 1))
        s.append(("k", p + 1))
        s.append(("max", p))
        s.append(("v", p + 1))
        s.append(("exp", p))
        if p >= LAG:
            s.append(("out", nout))
            nout += 1
        for _ in range(per):
            if bwork:
                s.append(bwork.pop(0))
        if p == BOUT:
            assert not bwork
            s.append(("bout",))
        if p == BLN:
            s.append(("bln",))
            s.append(("hln",))
    p = NP - 1
    s += [("qk", p), ("pv", p - 1)]
    rest = NP - nout
    before = rest - 2
    s.append(("out", nout)); nout += 1
    s.append(("max", p))
    if before >= 2:
        s.append(("out", nout)); nout += 1
    s.append(("exp", p))
    for _ in range(before - 2):
        s.append(("out", nout)); nout += 1
    s.append(("pv", p))
    s.append(("out", nout)); nout += 1
    s.append(("bproj", 0))
    s.append(("out", nout)); nout += 1
    assert nout == NP
    s.append(("bproj", 1))
    s.append(("xupd",))
    s.append(("bproj", 2))
    return s


def _kernel(x_hbm, mem0_ref, wqt_hbm, wkt_hbm, wvt_hbm, wo_hbm, bqkv_hbm, bwo_hbm,
            out_hbm,
            xs, w_s, wo_s, bqkv_s, bwo_s, hbuf, hbbuf, qbuf, kbuf, vbuf,
            x_st, q_st, k_st, v_st, o_st, bqkv_st, bwo_st, out_st, perm_s, permt_s, wsem, msem, osem,
            *, S, D, H, DH, M, SEG, W, DIL, HB):
    NSEG = S // SEG
    NG = 2 * NSEG
    L = M + SEG
    NP = H // 2
    PW = 2 * DH
    a_scale = _bf16_const(DH ** -0.5)
    b_scale = _bf16_const((D // HB) ** -0.5)
    TAIL = 16
    NT = D // 128

    OC = 256
    NOC = S // OC

    def wcopies(p):
        r = pl.ds(p * PW, PW)
        return [pltpu.make_async_copy(src.at[r, :], dst.at[r, :], wsem.at[i, p])
                for i, (src, dst) in enumerate(((wqt_hbm, q_st), (wkt_hbm, k_st), (wvt_hbm, v_st), (wo_hbm, o_st)))]

    def ocopy(c):
        r = pl.ds(c * OC, OC)
        return pltpu.make_async_copy(out_st.at[r, :], out_hbm.at[r, :], osem.at[0])

    X0 = 256
    misc = [pltpu.make_async_copy(bqkv_hbm, bqkv_st, msem.at[0]),
            pltpu.make_async_copy(bwo_hbm, bwo_st, msem.at[1]),
            pltpu.make_async_copy(x_hbm.at[0:X0, :], x_st.at[0:X0, :], msem.at[2]),
            pltpu.make_async_copy(x_hbm.at[X0:S, :], x_st.at[X0:S, :], msem.at[3])]
    misc[2].start()
    misc[0].start()
    misc[1].start()
    for p in range(AHEAD):
        for cp in wcopies(p):
            cp.start()
    if AHEAD >= NP:
        misc[3].start()

    kbuf[...] = jnp.zeros(kbuf.shape, F32)
    vbuf[...] = jnp.zeros(vbuf.shape, F32)
    qbuf[...] = jnp.zeros(qbuf.shape, F32)
    hbbuf[...] = jnp.zeros(hbbuf.shape, F32)
    mem0 = mem0_ref[...].astype(F32)

    DB = D // HB
    ri = lax.broadcasted_iota(jnp.int32, (D, D), 0)
    ci = lax.broadcasted_iota(jnp.int32, (D, D), 1)
    perm_s[...] = jnp.where(ri == (ci % HB) * DB + ci // HB, 1.0, 0.0).astype(BF16)
    permt_s[...] = jnp.where(ci == (ri % HB) * DB + ri // HB, 1.0, 0.0).astype(BF16)

    def cvt_x(lo, hi):
        for i in range(lo, hi, 128):
            xs[i:i + 128, :] = x_st[i:i + 128, :].astype(F32)

    misc[2].wait()
    cvt_x(0, X0)
    hbuf[...] = _layernorm(xs[0:SEG, :])
    misc[0].wait()
    misc[1].wait()

    def rows(seg):
        return pl.ds(pl.multiple_of(seg * SEG, SEG), SEG)

    def b_ln(seg):
        hbbuf[...] = _layernorm(xs[rows(seg), :])

    def b_proj(seg, j):
        y = _dot(hbbuf[...], _w(bqkv_s[:, j * D:(j + 1) * D]))
        if j == 0:
            qbuf[...] = y * b_scale
        else:
            buf = kbuf if j == 1 else vbuf
            buf[0:TAIL, :] = jnp.where(seg == 0, 0.0, buf[SEG:SEG + TAIL, :])
            buf[TAIL:, :] = y

    def b_logit(st, seg, w):
        off = TAIL - DIL * w
        s = None
        for j in range(NT):
            c = slice(j * 128, (j + 1) * 128)
            t = qbuf[:, c] * kbuf[off:off + SEG, c]
            s = t if s is None else s + t
        s = s + pltpu.roll(s, 64, 1)
        s = s + pltpu.roll(s, 32, 1)
        if w > 0:
            pos = lax.broadcasted_iota(jnp.int32, (SEG, 128), 0) + seg * SEG
            s = jnp.where(pos >= DIL * w, s, NEG)
        st.setdefault("blog", []).append(s)

    def b_softmax(st):
        logits = st["blog"]
        m = functools.reduce(jnp.maximum, logits)
        es = [jnp.exp(s - m) for s in logits]
        st["bexp"] = es
        st["binv"] = _recip(functools.reduce(jnp.add, es))

    def b_pv(st, j):
        c = slice(j * 128, (j + 1) * 128)
        oj = None
        for w in range(W):
            off = TAIL - DIL * w
            t = st["bexp"][w] * vbuf[off:off + SEG, c]
            oj = t if oj is None else oj + t
        st.setdefault("bo", []).append(oj * st["binv"])

    def b_out(st, seg, active):
        o = jnp.concatenate(st["bo"], axis=1)
        x1 = xs[rows(seg), :]
        x2 = x1 + _dot(o, _w(bwo_s[...]))
        x2 = jnp.where(active, x2, x1)
        xs[rows(seg), :] = x2
        out_st[rows(seg), :] = x2.astype(out_st.dtype)

    def a_proj(st, p, j, pw=None):
        pw = p if pw is None else pw
        st["qkv"[j], p] = _dot(st["h"], _w(w_s[pw, :, j * PW:(j + 1) * PW]))

    def _split_heads(t):
        lane = lax.broadcasted_iota(jnp.int32, (L, 128), 1)
        lo = lane < (DH - 128)
        z = jnp.zeros((L, 128), F32)
        t0, t1, t2 = t[:, 0:128], t[:, 128:256], t[:, 256:384]
        top = jnp.concatenate([t0, jnp.where(lo, t1, 0.0), z], axis=1)
        bot = jnp.concatenate([z, jnp.where(lo, 0.0, t1), t2], axis=1)
        return jnp.concatenate([top, bot], axis=0).astype(BF16)

    def a_qk(st, p):
        st["s", p] = _dot_nt(st["q", p], _split_heads(st["k", p]))

    def _smask():
        row = lax.broadcasted_iota(jnp.int32, (L, 2 * L), 0)
        col = lax.broadcasted_iota(jnp.int32, (L, 2 * L), 1)
        lo = col < L
        key = jnp.where(lo, col, col - L)
        return lo, (row < M) | (row >= key)

    def a_max(st, p):
        lo, mask = _smask()
        s = jnp.where(mask, st["s", p] * a_scale, NEG)
        m_lo = jnp.max(jnp.where(lo, s, -jnp.inf), axis=-1, keepdims=True)
        m_hi = jnp.max(jnp.where(lo, -jnp.inf, s), axis=-1, keepdims=True)
        st["s", p] = s
        st["m", p] = (m_lo, m_hi)

    def a_exp(st, p):
        lo, _ = _smask()
        m_lo, m_hi = st["m", p]
        e = jnp.exp(st["s", p] - jnp.where(lo, m_lo, m_hi))
        d_lo = jnp.sum(jnp.where(lo, e, 0.0), axis=-1, keepdims=True)
        d_hi = jnp.sum(jnp.where(lo, 0.0, e), axis=-1, keepdims=True)
        st["e", p] = e
        st["d", p] = (d_lo, d_hi)

    def a_pv(st, p):
        lo, _ = _smask()
        d_lo, d_hi = st["d", p]
        pr = st["e", p] * _recip(jnp.where(lo, d_lo, d_hi))
        st["o", p] = _dot(pr, _split_heads(st["v", p]))

    def a_out(st, p, pw=None):
        y = _dot(st["o", p], _w(wo_s[p if pw is None else pw]))
        st["acc"] = y if "acc" not in st else st["acc"] + y

    def first_pair(p, acc):
        @pl.when(p + AHEAD < NP)
        def _():
            for cp in wcopies(jnp.minimum(p + AHEAD, NP - 1)):
                cp.start()

        if AHEAD < NP:
            @pl.when(p + AHEAD == NP)
            def _():
                misc[3].start()

        @pl.when(p < 3 * NT)
        def _():
            blk = pl.ds(pl.multiple_of((p // NT) * D, 128), D)
            til = pl.ds(pl.multiple_of((p % NT) * 128, 128), 128)
            dst = pl.ds(pl.multiple_of(p * 128, 128), 128)
            bqkv_s[:, dst] = pltpu.bitcast(_dot(bqkv_st[:, blk], perm_s[:, til]).astype(BF16), U32)

        @pl.when(p < NT)
        def _():
            til = pl.ds(pl.multiple_of(p * 128, 128), 128)
            bwo_s[:, til] = pltpu.bitcast(_dot(permt_s[...], bwo_st[:, til]).astype(BF16), U32)

        r = pl.ds(pl.multiple_of(p * PW, PW), PW)
        cps = wcopies(p)
        for cp in cps:
            cp.wait()
        for j, st_ref in enumerate((q_st, k_st, v_st)):
            w_s[p, :, j * PW:(j + 1) * PW] = pltpu.bitcast(st_ref[r, :].T, U32)
        wo_s[p] = pltpu.bitcast(o_st[r, :], U32)
        st = {"h": jnp.concatenate([mem0, hbuf[...]], axis=0), "acc": acc}
        for j in range(3):
            a_proj(st, 0, j, p)
        a_qk(st, 0)
        a_max(st, 0)
        a_exp(st, 0)
        a_pv(st, 0)
        a_out(st, 0, p)
        return st["acc"]

    acc0 = lax.fori_loop(0, NP, first_pair, jnp.zeros((L, D), F32))
    xs[0:SEG, :] = xs[0:SEG, :] + acc0[M:, :]
    hbuf[...] = _layernorm(xs[SEG:2 * SEG, :])

    def step(g, mem):
        seg = g % NSEG
        seg1 = (g + NSEG - 1) % NSEG
        seg2 = (g + NSEG - 2) % NSEG
        segn = (g + 1) % NSEG
        mem = jnp.where(seg == 0, mem0, mem)
        first_out = NSEG + OC // SEG + 2

        @pl.when((g >= first_out) & ((g - first_out) % (OC // SEG) == 0))
        def _():
            ocopy((g - first_out) // (OC // SEG)).start()
        st = {"h": jnp.concatenate([mem, hbuf[...]], axis=0)}

        sched = build_schedule(NP)
        for item in sched:
            op, arg = item[0], item[1:]
            if op in "qkv" and len(op) == 1:
                a_proj(st, arg[0], "qkv".index(op))
            elif op == "qk":
                a_qk(st, arg[0])
            elif op == "max":
                a_max(st, arg[0])
            elif op == "exp":
                a_exp(st, arg[0])
            elif op == "pv":
                a_pv(st, arg[0])
            elif op == "out":
                a_out(st, arg[0])
            elif op == "blog":
                b_logit(st, seg2, arg[0])
            elif op == "bsm":
                b_softmax(st)
            elif op == "bpv":
                b_pv(st, arg[0])
            elif op == "bout":
                b_out(st, seg2, g >= 2)
            elif op == "bln":
                b_ln(seg1)
            elif op == "bproj":
                b_proj(seg1, arg[0])
            elif op == "xupd":
                xs[rows(seg), :] = xs[rows(seg), :] + st["acc"][M:, :]
            elif op == "hln":
                hbuf[...] = _layernorm(xs[rows(segn), :])
            else:
                raise ValueError(op)
        return st["acc"][:M, :]


    NB = (NG - 2) // UNROLL
    assert NB * UNROLL == NG - 2

    def body(i, mem):
        @pl.when(i == 1)
        def _():
            misc[3].wait()
            cvt_x(X0, S)
        for u in range(UNROLL):
            mem = step(1 + i * UNROLL + u, mem)
        return mem

    mem = lax.fori_loop(0, NB, body, acc0[:M, :])
    step(NG - 1, mem)

    for i, seg in enumerate((NSEG - 2, NSEG - 1)):
        st = {}
        for w in range(W):
            b_logit(st, seg, w)
        b_softmax(st)
        for j in range(NT):
            b_pv(st, j)
        if i == 0:
            b_ln(NSEG - 1)
        b_out(st, seg, True)
        if i == 0:
            for j in range(3):
                b_proj(NSEG - 1, j)
    ocopy(NOC - 1).start()
    for c in range(NOC):
        ocopy(c).wait()


@functools.partial(jax.jit, static_argnames=("A_seg_len",))
def pallas_interleave_layers__memory_aug_recurrent_mem_tr__sliding_local_dilated__prompt_kernel(A_x, A_mem0, A_Wq, A_Wk, A_Wv, A_Wo, A_seg_len, B_x, B_wqkv, B_wo):
    del B_x
    B, S, D = A_x.shape
    M = A_mem0.shape[1]
    _, H, DH = A_Wq.shape
    SEG = int(A_seg_len)
    HB, W, DIL = 32, 8, 2
    DB = D // HB
    x2 = A_x.reshape(S, D)
    mem0 = A_mem0.reshape(M, D)
    wq = A_Wq.transpose(1, 2, 0).reshape(H * DH, D)
    wk = A_Wk.transpose(1, 2, 0).reshape(H * DH, D)
    wv = A_Wv.transpose(1, 2, 0).reshape(H * DH, D)
    wo = A_Wo.reshape(H * DH, D)
    bqkv, bwo = B_wqkv, B_wo
    NP = H // 2
    hbm = pl.BlockSpec(memory_space=pl.ANY)
    out = pl.pallas_call(
        functools.partial(_kernel, S=S, D=D, H=H, DH=DH, M=M, SEG=SEG, W=W, DIL=DIL, HB=HB),
        out_shape=jax.ShapeDtypeStruct((S, D), A_x.dtype),
        in_specs=[hbm, pl.BlockSpec(memory_space=pltpu.VMEM), hbm, hbm, hbm, hbm, hbm, hbm],
        out_specs=hbm,
        scratch_shapes=[
            pltpu.VMEM((S, D), F32),
            pltpu.VMEM((NP, D // 2, 6 * DH), U32),
            pltpu.VMEM((NP, DH, D), U32),
            pltpu.VMEM((D // 2, 3 * D), U32),
            pltpu.VMEM((D // 2, D), U32),
            pltpu.VMEM((SEG, D), F32),
            pltpu.VMEM((SEG, D), F32),
            pltpu.VMEM((SEG, D), F32),
            pltpu.VMEM((16 + SEG, D), F32),
            pltpu.VMEM((16 + SEG, D), F32),
            pltpu.VMEM((S, D), BF16),
            pltpu.VMEM((H * DH, D), BF16),
            pltpu.VMEM((H * DH, D), BF16),
            pltpu.VMEM((H * DH, D), BF16),
            pltpu.VMEM((H * DH, D), BF16),
            pltpu.VMEM((D, 3 * D), BF16),
            pltpu.VMEM((D, D), BF16),
            pltpu.VMEM((S, D), BF16),
            pltpu.VMEM((D, D), BF16),
            pltpu.VMEM((D, D), BF16),
            pltpu.SemaphoreType.DMA((4, NP)),
            pltpu.SemaphoreType.DMA((4,)),
            pltpu.SemaphoreType.DMA((1,)),
        ],
        compiler_params=pltpu.CompilerParams(vmem_limit_bytes=120 * 1024 * 1024),
    )(x2, mem0, wq, wk, wv, wo, bqkv, bwo)
    return out.reshape(B, S, D)
```

```python
import functools

import jax
import jax.numpy as jnp
import numpy as np
from jax import lax
from jax.experimental import pallas as pl
from jax.experimental.pallas import tpu as pltpu

F32 = jnp.float32
BF16 = jnp.bfloat16
U32 = jnp.uint32
NEG = -1000000000.0
OUT_LAG = 2
UA = 3
UB = 2
AHEAD = 2


def _bf16_const(v):
    return float(np.asarray(v, dtype=BF16).astype(np.float32))


def _dot(a, b):
    return lax.dot_general(a, b, (((1,), (0,)), ((), ())), preferred_element_type=F32)


def _dot_nt(a, b):
    return lax.dot_general(a, b, (((1,), (1,)), ((), ())), preferred_element_type=F32)


def _layernorm(x):
    m = jnp.mean(x, axis=-1, keepdims=True)
    c = x - m
    v = jnp.mean(c * c, axis=-1, keepdims=True)
    return c * lax.rsqrt(v + 1e-5)


def _w(ref_slice):
    return pltpu.bitcast(ref_slice, BF16)


def _recip(d):
    r = pl.reciprocal(d, approx=True)
    return r * (2.0 - d * r)


LAG = 5
NPRE = 36
PR = 8
PADPV = 1
BOUT = 9
BLN = 12


def build_schedule(NP):
    s = [("q", 0), ("k", 0), ("v", 0)]
    bwork = [("blog", w) for w in range(8)] + [("bsm",)] + [("bpv", j) for j in range(5)]
    per = -(-len(bwork) // BOUT)
    nout = 0
    for p in range(NP):
        nxt = p + 1 < NP
        if not nxt:
            break
        s.append(("q", p + 1))
        s.append(("qk", p))
        if p >= 1:
            s.append(("pv", p - 1))
        s.append(("k", p + 1))
        s.append(("max", p))
        s.append(("v", p + 1))
        s.append(("exp", p))
        if p >= LAG:
            s.append(("out", nout))
            nout += 1
        for _ in range(per):
            if bwork:
                s.append(bwork.pop(0))
        if p == BOUT:
            assert not bwork
            s.append(("bout",))
        if p == BLN:
            s.append(("bln",))
            s.append(("hln",))
    p = NP - 1
    s += [("qk", p), ("pv", p - 1)]
    rest = NP - nout
    before = rest - 2
    s.append(("out", nout)); nout += 1
    s.append(("max", p))
    if before >= 2:
        s.append(("out", nout)); nout += 1
    s.append(("exp", p))
    for _ in range(before - 2):
        s.append(("out", nout)); nout += 1
    s.append(("pv", p))
    s.append(("out", nout)); nout += 1
    s.append(("bproj", 0))
    s.append(("out", nout)); nout += 1
    assert nout == NP
    s.append(("bproj", 1))
    s.append(("xupd",))
    s.append(("bproj", 2))
    return s


def _kernel(x_hbm, mem0_ref, wqt_hbm, wkt_hbm, wvt_hbm, wo_hbm, bqkv_hbm, bwo_hbm,
            out_hbm,
            xs, w_s, wo_s, bqkv_s, bwo_s, hbuf, hbbuf, qbuf, kbuf, vbuf,
            x_st, q_st, k_st, v_st, o_st, bqkv_st, bwo_st, out_st, g_s, xp_st, hall_s, pre_s,
            wsem, bsem, msem, osem,
            *, S, D, H, DH, M, SEG, W, DIL, HB):
    NSEG = S // SEG
    NG = 2 * NSEG
    L = M + SEG
    NP = H // 2
    PW = 2 * DH
    a_scale = _bf16_const(DH ** -0.5)
    b_scale = _bf16_const((D // HB) ** -0.5)
    TAIL = 16
    NT = D // 128

    OC = 256
    NOC = S // OC

    def wcopies(p):
        r = pl.ds(p * PW, PW)
        return [pltpu.make_async_copy(src.at[r, :], dst.at[r, :], wsem.at[i, p])
                for i, (src, dst) in enumerate(((wqt_hbm, q_st), (wkt_hbm, k_st), (wvt_hbm, v_st), (wo_hbm, o_st)))]

    def ocopy(c):
        r = pl.ds(c * OC, OC)
        return pltpu.make_async_copy(out_st.at[r, :], out_hbm.at[r, :], osem.at[0])

    X0 = 256 // SEG
    cp_x0 = pltpu.make_async_copy(x_hbm.at[0:X0], x_st.at[0:X0], msem.at[0])
    cp_x1 = pltpu.make_async_copy(x_hbm.at[X0:NSEG], x_st.at[X0:NSEG], msem.at[1])
    cp_xp = pltpu.make_async_copy(x_hbm.at[1:NPRE + 1, SEG - PR:SEG, :], xp_st, msem.at[2])
    cp_bo = pltpu.make_async_copy(bwo_hbm, bwo_st, msem.at[3])
    NU = 3 * NT

    def bcopy(u):
        r = pl.ds(pl.multiple_of((u % NT) * 128, 128), 128)
        c = pl.ds(pl.multiple_of((u // NT) * D, 128), D)
        return pltpu.make_async_copy(bqkv_hbm.at[r, c], bqkv_st.at[r, c], bsem.at[u])

    cp_x0.start()
    cp_xp.start()
    for cp in wcopies(0):
        cp.start()
    bcopy(0).start()

    kbuf[...] = jnp.zeros(kbuf.shape, F32)
    vbuf[...] = jnp.zeros(vbuf.shape, F32)
    qbuf[...] = jnp.zeros(qbuf.shape, F32)
    hbbuf[...] = jnp.zeros(hbbuf.shape, F32)
    mem0 = mem0_ref[...].astype(F32)

    DB = D // HB

    def cvt_x(lo, hi):
        for i in range(lo, hi):
            xs[i * SEG:(i + 1) * SEG, :] = x_st[i].astype(F32)

    def rows(seg):
        return pl.ds(pl.multiple_of(seg * SEG, SEG), SEG)

    def b_ln(seg):
        hbbuf[...] = _layernorm(xs[rows(seg), :])

    def b_proj(seg, j):
        y = _dot(hbbuf[...], _w(bqkv_s[:, j * D:(j + 1) * D]))
        if j == 0:
            qbuf[...] = y * b_scale
        else:
            buf = kbuf if j == 1 else vbuf
            buf[0:TAIL, :] = jnp.where(seg == 0, 0.0, buf[SEG:SEG + TAIL, :])
            buf[TAIL:, :] = y

    def b_logit(st, seg, w):
        off = TAIL - DIL * w
        s = None
        for j in range(NT):
            c = slice(j * 128, (j + 1) * 128)
            t = qbuf[:, c] * kbuf[off:off + SEG, c]
            s = t if s is None else s + t
        s = s + pltpu.roll(s, 64, 1)
        s = s + pltpu.roll(s, 32, 1)
        if w > 0:
            pos = lax.broadcasted_iota(jnp.int32, (SEG, 128), 0) + seg * SEG
            s = jnp.where(pos >= DIL * w, s, NEG)
        st.setdefault("blog", []).append(s)

    def b_softmax(st):
        logits = st["blog"]
        m = functools.reduce(jnp.maximum, logits)
        es = [jnp.exp(s - m) for s in logits]
        st["bexp"] = es
        st["binv"] = _recip(functools.reduce(jnp.add, es))

    def b_pv(st, j):
        c = slice(j * 128, (j + 1) * 128)
        oj = None
        for w in range(W):
            off = TAIL - DIL * w
            t = st["bexp"][w] * vbuf[off:off + SEG, c]
            oj = t if oj is None else oj + t
        st.setdefault("bo", []).append(oj * st["binv"])

    def b_out(st, seg, active):
        o = jnp.concatenate(st["bo"], axis=1)
        x1 = xs[rows(seg), :]
        x2 = x1 + _dot(o, _w(bwo_s[...]))
        x2 = jnp.where(active, x2, x1)
        xs[rows(seg), :] = x2
        out_st[rows(seg), :] = x2.astype(out_st.dtype)

    def a_proj(st, p, j, pw=None):
        pw = p if pw is None else pw
        y = _dot(st["h"], _w(w_s[pw, :, j * PW:(j + 1) * PW]))
        if "pre" in st:
            y = jnp.concatenate([y, pre_s[p, st["pre"], j * PW:(j + 1) * PW]], axis=0)
        st["qkv"[j], p] = y

    def _split_heads(t):
        lane = lax.broadcasted_iota(jnp.int32, (L, 128), 1)
        lo = lane < (DH - 128)
        z = jnp.zeros((L, 128), F32)
        t0, t1, t2 = t[:, 0:128], t[:, 128:256], t[:, 256:384]
        top = jnp.concatenate([t0, jnp.where(lo, t1, 0.0), z], axis=1)
        bot = jnp.concatenate([z, jnp.where(lo, 0.0, t1), t2], axis=1)
        return jnp.concatenate([top, bot], axis=0).astype(BF16)

    def a_qk(st, p):
        st["s", p] = _dot_nt(st["q", p], _split_heads(st["k", p]))

    def _smask():
        row = lax.broadcasted_iota(jnp.int32, (L, 128), 0)
        col = lax.broadcasted_iota(jnp.int32, (L, 128), 1)
        lo = col < L
        key = jnp.where(lo, col, col - L)
        visible = ((row < M) | (row >= key)) & (col < 2 * L)
        fill = jnp.where(col < 2 * L, NEG, -jnp.inf)
        return lo, visible, fill

    def a_max(st, p):
        lo, visible, fill = _smask()
        s = jnp.concatenate([st["s", p], jnp.zeros((L, 128 - 2 * L), F32)], axis=1)
        s = jnp.where(visible, s * a_scale, fill)
        m_lo = jnp.max(jnp.where(lo, s, -jnp.inf), axis=-1, keepdims=True)
        m_hi = jnp.max(jnp.where(lo, -jnp.inf, s), axis=-1, keepdims=True)
        st["s", p] = s
        st["m", p] = (m_lo, m_hi)

    def a_exp(st, p):
        lo = _smask()[0]
        m_lo, m_hi = st["m", p]
        e = jnp.exp(st["s", p] - jnp.where(lo, m_lo, m_hi))
        d_lo = jnp.sum(jnp.where(lo, e, 0.0), axis=-1, keepdims=True)
        d_hi = jnp.sum(jnp.where(lo, 0.0, e), axis=-1, keepdims=True)
        st["e", p] = e
        st["d", p] = (d_lo, d_hi)

    def a_norm(st, p):
        lo = _smask()[0]
        d_lo, d_hi = st["d", p]
        vb = jnp.concatenate([_split_heads(st["v", p]), jnp.zeros((128 - 2 * L, PW), BF16)], axis=0)
        return st["e", p] * _recip(jnp.where(lo, d_lo, d_hi)), vb

    def pv_dot(pr, vb):
        return _dot(pr, vb)

    def a_pv(st, p):
        st["o", p] = pv_dot(*a_norm(st, p))

    def a_out(st, p, pw=None):
        y = _dot(st["o", p], _w(wo_s[p if pw is None else pw]))
        st["acc"] = y if "acc" not in st else st["acc"] + y

    def gather_heads(t):
        return jnp.concatenate(
            [g_s[pl.ds(4 * t + dd, HB, stride=DB), :] for dd in range(128 // HB)], axis=0)

    def perm_unit(u):
        j, a = u // NT, u % NT
        r = pl.ds(pl.multiple_of(a * 128, 128), 128)
        for f in range(NT):
            c = pl.ds(pl.multiple_of(j * D + f * 128, 128), 128)
            g_s[f * 128:(f + 1) * 128, :] = bqkv_st[r, c].astype(F32).T
        for t in range(NT):
            c = pl.ds(pl.multiple_of(j * D + t * 128, 128), 128)
            bqkv_s[pl.ds(pl.multiple_of(a * 64, 64), 64), c] = pltpu.bitcast(
                gather_heads(t).T.astype(BF16), U32)

    def perm_wo():
        for f in range(NT):
            c = slice(f * 128, (f + 1) * 128)
            g_s[...] = bwo_st[:, c].astype(F32)
            for t in range(NT):
                bwo_s[t * 64:(t + 1) * 64, c] = pltpu.bitcast(gather_heads(t).astype(BF16), U32)

    cp_x0.wait()
    for p in range(1, AHEAD):
        for cp in wcopies(p):
            cp.start()
        bcopy(p).start()
    cvt_x(0, X0)
    cp_xp.wait()
    hall_s[0:M, :] = mem0
    hall_s[M:L, :] = _layernorm(xs[0:SEG, :])
    hall_s[L:, :] = _layernorm(xp_st[...].astype(F32).reshape(NPRE * PR, D))

    def first_pair(p, carry):
        acc, pr_prev, vb_prev = carry

        r = pl.ds(pl.multiple_of(p * PW, PW), PW)
        rprev = pl.ds(pl.multiple_of(jnp.maximum(p - 1, 0) * PW, PW), PW)
        for cp in wcopies(p):
            cp.wait()

        @pl.when(p < NU)
        def _():
            bcopy(jnp.minimum(p, NU - 1)).wait()

        @pl.when(p + AHEAD < NP)
        def _():
            for cp in wcopies(jnp.minimum(p + AHEAD, NP - 1)):
                cp.start()

        @pl.when(p + AHEAD < NU)
        def _():
            bcopy(jnp.minimum(p + AHEAD, NU - 1)).start()

        @pl.when(p + AHEAD == NP)
        def _():
            cp_bo.start()
            cp_x1.start()

        st = {}

        def proj(j):
            src = (q_st, k_st, v_st)[j]
            y = _dot_nt(hall_s[...], src[r, :])
            st["qkv"[j], 0] = y[:L, :]
            pre_s[p, :, j * PW:(j + 1) * PW] = y[L:, :]

        def repack(j):
            src = (q_st, k_st, v_st)[j]
            w_s[p, :, j * PW:(j + 1) * PW] = pltpu.bitcast(src[r, :].T, U32)

        proj(0)
        o_prev = _dot(pr_prev, vb_prev)
        proj(1)
        acc = acc + _dot(o_prev, o_st[rprev, :])
        a_qk(st, 0)
        repack(0)
        proj(2)
        a_max(st, 0)
        perm_unit(jnp.minimum(p, NU - 1))
        repack(1)
        a_exp(st, 0)
        repack(2)
        wo_s[p] = pltpu.bitcast(o_st[r, :], U32)
        pr, vb = a_norm(st, 0)
        return acc, pr, vb

    acc0, pr, vb = lax.fori_loop(
        0, NP, first_pair,
        (jnp.zeros((L, D), F32), jnp.zeros((L, 128), F32), jnp.zeros((128, PW), BF16)))
    cp_bo.wait()
    acc0 = acc0 + _dot(_dot(pr, vb), o_st[(NP - 1) * PW:NP * PW, :])
    perm_wo()
    xs[0:SEG, :] = xs[0:SEG, :] + acc0[M:, :]
    hbuf[...] = _layernorm(xs[SEG:2 * SEG, :])

    def step(g, mem, pre=False):
        seg = g % NSEG
        seg1 = (g + NSEG - 1) % NSEG
        seg2 = jnp.maximum(g - 2, 0) % NSEG
        segn = (g + 1) % NSEG
        mem = jnp.where(seg == 0, mem0, mem)
        first_out = NSEG + OC // SEG + 2

        @pl.when((g >= first_out) & ((g - first_out) % (OC // SEG) == 0))
        def _():
            ocopy((g - first_out) // (OC // SEG)).start()
        if pre:
            st = {"h": jnp.concatenate([mem, hbuf[0:SEG - PR, :]], axis=0),
                  "pre": pl.ds(pl.multiple_of((g - 1) * PR, PR), PR)}
        else:
            st = {"h": jnp.concatenate([mem, hbuf[...]], axis=0)}

        sched = build_schedule(NP)
        for item in sched:
            op, arg = item[0], item[1:]
            if op in "qkv" and len(op) == 1:
                a_proj(st, arg[0], "qkv".index(op))
            elif op == "qk":
                a_qk(st, arg[0])
            elif op == "max":
                a_max(st, arg[0])
            elif op == "exp":
                a_exp(st, arg[0])
            elif op == "pv":
                a_pv(st, arg[0])
            elif op == "out":
                a_out(st, arg[0])
            elif op == "blog":
                b_logit(st, seg2, arg[0])
            elif op == "bsm":
                b_softmax(st)
            elif op == "bpv":
                b_pv(st, arg[0])
            elif op == "bout":
                b_out(st, seg2, g >= 2)
            elif op == "bln":
                b_ln(seg1)
            elif op == "bproj":
                b_proj(seg1, arg[0])
            elif op == "xupd":
                xs[rows(seg), :] = xs[rows(seg), :] + st["acc"][M:, :]
            elif op == "hln":
                hbuf[...] = _layernorm(xs[rows(segn), :])
            else:
                raise ValueError(op)
        return st["acc"][:M, :]


    assert NPRE % UA == 0 and (NG - 2 - NPRE) % UB == 0 and NPRE >= X0 and NPRE < NSEG
    assert 3 * NT <= NP - 1

    def body_pre(i, mem):
        @pl.when(i == (X0 - 2) // UA)
        def _():
            cp_x1.wait()
            cvt_x(X0, NSEG)
        for u in range(UA):
            mem = step(1 + i * UA + u, mem, pre=True)
        return mem

    def body(i, mem):
        for u in range(UB):
            mem = step(1 + NPRE + i * UB + u, mem)
        return mem

    mem = lax.fori_loop(0, NPRE // UA, body_pre, acc0[:M, :])
    mem = lax.fori_loop(0, (NG - 2 - NPRE) // UB, body, mem)
    step(NG - 1, mem)

    for i, seg in enumerate((NSEG - 2, NSEG - 1)):
        st = {}
        for w in range(W):
            b_logit(st, seg, w)
        b_softmax(st)
        for j in range(NT):
            b_pv(st, j)
        if i == 0:
            b_ln(NSEG - 1)
        b_out(st, seg, True)
        if i == 0:
            for j in range(3):
                b_proj(NSEG - 1, j)
    ocopy(NOC - 1).start()
    for c in range(NOC):
        ocopy(c).wait()


@functools.partial(jax.jit, static_argnames=("A_seg_len",))
def pallas_interleave_layers__memory_aug_recurrent_mem_tr__sliding_local_dilated__prompt_kernel(A_x, A_mem0, A_Wq, A_Wk, A_Wv, A_Wo, A_seg_len, B_x, B_wqkv, B_wo):
    del B_x
    B, S, D = A_x.shape
    M = A_mem0.shape[1]
    _, H, DH = A_Wq.shape
    SEG = int(A_seg_len)
    HB, W, DIL = 32, 8, 2
    DB = D // HB
    x2 = A_x.reshape(S // SEG, SEG, D)
    mem0 = A_mem0.reshape(M, D)
    wq = A_Wq.transpose(1, 2, 0).reshape(H * DH, D)
    wk = A_Wk.transpose(1, 2, 0).reshape(H * DH, D)
    wv = A_Wv.transpose(1, 2, 0).reshape(H * DH, D)
    wo = A_Wo.reshape(H * DH, D)
    bqkv, bwo = B_wqkv, B_wo
    NP = H // 2
    hbm = pl.BlockSpec(memory_space=pl.ANY)
    out = pl.pallas_call(
        functools.partial(_kernel, S=S, D=D, H=H, DH=DH, M=M, SEG=SEG, W=W, DIL=DIL, HB=HB),
        out_shape=jax.ShapeDtypeStruct((S, D), A_x.dtype),
        in_specs=[hbm, pl.BlockSpec(memory_space=pltpu.VMEM), hbm, hbm, hbm, hbm, hbm, hbm],
        out_specs=hbm,
        scratch_shapes=[
            pltpu.VMEM((S, D), F32),
            pltpu.VMEM((NP, D // 2, 6 * DH), U32),
            pltpu.VMEM((NP, DH, D), U32),
            pltpu.VMEM((D // 2, 3 * D), U32),
            pltpu.VMEM((D // 2, D), U32),
            pltpu.VMEM((SEG, D), F32),
            pltpu.VMEM((SEG, D), F32),
            pltpu.VMEM((SEG, D), F32),
            pltpu.VMEM((16 + SEG, D), F32),
            pltpu.VMEM((16 + SEG, D), F32),
            pltpu.VMEM((S // SEG, SEG, D), BF16),
            pltpu.VMEM((H * DH, D), BF16),
            pltpu.VMEM((H * DH, D), BF16),
            pltpu.VMEM((H * DH, D), BF16),
            pltpu.VMEM((H * DH, D), BF16),
            pltpu.VMEM((D, 3 * D), BF16),
            pltpu.VMEM((D, D), BF16),
            pltpu.VMEM((S, D), BF16),
            pltpu.VMEM((D, 128), F32),
            pltpu.VMEM((NPRE, PR, D), BF16),
            pltpu.VMEM((M + SEG + NPRE * PR, D), F32),
            pltpu.VMEM((NP, NPRE * PR, 6 * DH), F32),
            pltpu.SemaphoreType.DMA((4, NP)),
            pltpu.SemaphoreType.DMA((3 * D // 128,)),
            pltpu.SemaphoreType.DMA((4,)),
            pltpu.SemaphoreType.DMA((1,)),
        ],
        compiler_params=pltpu.CompilerParams(vmem_limit_bytes=120 * 1024 * 1024),
    )(x2, mem0, wq, wk, wv, wo, bqkv, bwo)
    return out.reshape(B, S, D)
```

```python
import functools

import jax
import jax.numpy as jnp
import numpy as np
from jax import lax
from jax.experimental import pallas as pl
from jax.experimental.pallas import tpu as pltpu

F32 = jnp.float32
BF16 = jnp.bfloat16
U32 = jnp.uint32
NEG = -1000000000.0

NPRE = 36
PR = 8
UNROLL = 2
OUT_LAG = 6
B_OUT_AT = 7
LN_AT = 12


def _bf16_const(v):
    return float(np.asarray(v, dtype=BF16).astype(np.float32))


def _dot(a, b):
    return lax.dot_general(a, b, (((1,), (0,)), ((), ())), preferred_element_type=F32)


def _dot_nt(a, b):
    return lax.dot_general(a, b, (((1,), (1,)), ((), ())), preferred_element_type=F32)


def _layernorm(x):
    m = jnp.mean(x, axis=-1, keepdims=True)
    c = x - m
    v = jnp.mean(c * c, axis=-1, keepdims=True)
    return c * lax.rsqrt(v + 1e-5)


def _pack(x):
    return pltpu.bitcast(x, U32)


def _unpack(x):
    return pltpu.bitcast(x, BF16)


def _recip(d):
    r = pl.reciprocal(d, approx=True)
    return r * (2.0 - d * r)


def _schedule(n_pairs, n_window, n_tiles):
    s = [("q", 0), ("k", 0), ("v", 0)]
    bwork = ([("blog", w) for w in range(n_window)] + [("bsm",)]
             + [("bpv", j) for j in range(n_tiles)])
    per_slot = -(-len(bwork) // B_OUT_AT)
    n_out = 0
    for p in range(n_pairs - 1):
        s += [("q", p + 1), ("qk", p)]
        if p >= 1:
            s.append(("pv", p - 1))
        s += [("k", p + 1), ("max", p), ("v", p + 1), ("exp", p)]
        if p >= OUT_LAG:
            s.append(("out", n_out))
            n_out += 1
        for _ in range(per_slot):
            if bwork:
                s.append(bwork.pop(0))
        if p == B_OUT_AT:
            assert not bwork
            s.append(("bout",))
        if p == LN_AT - 2:
            s.append(("xcvt",))
        if p == LN_AT:
            s += [("bln",), ("hln",)]
    p = n_pairs - 1
    outs = [("out", i) for i in range(n_out, n_pairs)]
    s += [("qk", p), ("pv", p - 1), outs[0], ("max", p), outs[1], ("exp", p)]
    s += outs[2:-2]
    s += [("pv", p), outs[-2], ("bproj", 0), outs[-1], ("bproj", 1), ("xupd",), ("bproj", 2)]
    return s


def _kernel(x_hbm, mem0_ref, wqt_hbm, wkt_hbm, wvt_hbm, wo_hbm, bqkv_hbm, bwo_hbm,
            out_hbm,
            xs, w_s, wo_s, bqkv_s, bwo_s, hbuf, hbbuf, qbuf, kbuf, vbuf,
            x_st, q_st, k_st, v_st, o_st, bqkv_st, bwo_st, out_st, g_s, xp_st, hall_s, pre_s,
            wsem, bsem, msem, osem,
            *, S, D, H, DH, M, SEG, W, DIL, HB):
    NSEG = S // SEG
    NG = 2 * NSEG
    L = M + SEG
    NP = H // 2
    PW = 2 * DH
    NT = D // 128
    DB = D // HB
    NU = 3 * NT
    TAIL = 16
    OC = 256
    NOC = S // OC
    X0 = 256 // SEG
    a_scale = _bf16_const(DH ** -0.5)
    b_scale = _bf16_const(DB ** -0.5)
    assert DIL * (W - 1) <= TAIL and 128 % HB == 0 and NU <= NP - 1

    def wcopies(p):
        r = pl.ds(p * PW, PW)
        return [pltpu.make_async_copy(src.at[r, :], dst.at[r, :], wsem.at[i, p])
                for i, (src, dst) in enumerate(
                    ((wqt_hbm, q_st), (wkt_hbm, k_st), (wvt_hbm, v_st), (wo_hbm, o_st)))]

    def bcopy(u):
        r = pl.ds(pl.multiple_of((u % NT) * 128, 128), 128)
        c = pl.ds(pl.multiple_of((u // NT) * D, 128), D)
        return pltpu.make_async_copy(bqkv_hbm.at[r, c], bqkv_st.at[r, c], bsem.at[u])

    def ocopy(lo, hi):
        return pltpu.make_async_copy(out_st.at[pl.ds(lo, hi - lo), :],
                                     out_hbm.at[pl.ds(lo, hi - lo), :], osem.at[0])

    cp_x0 = pltpu.make_async_copy(x_hbm.at[0:2], x_st.at[0:2], msem.at[0])
    cp_x0b = pltpu.make_async_copy(x_hbm.at[2:X0], x_st.at[2:X0], msem.at[1])
    cp_x1 = pltpu.make_async_copy(x_hbm.at[X0:NSEG], x_st.at[X0:NSEG], msem.at[2])
    cp_xp = pltpu.make_async_copy(x_hbm.at[1:NPRE + 1, SEG - PR:SEG, :], xp_st, msem.at[3])
    cp_bo = pltpu.make_async_copy(bwo_hbm, bwo_st, msem.at[4])
    cp_q0, cp_k0, cp_v0, cp_o0 = wcopies(0)

    def rows(seg):
        return pl.ds(pl.multiple_of(seg * SEG, SEG), SEG)

    def gather_heads(t):
        n = 128 // HB
        return jnp.concatenate(
            [g_s[pl.ds(n * t + dd, HB, stride=DB), :] for dd in range(n)], axis=0)

    def perm_wqkv_piece(u):
        j, a = u // NT, u % NT
        r = pl.ds(pl.multiple_of(a * 128, 128), 128)
        for f in range(NT):
            c = pl.ds(pl.multiple_of(j * D + f * 128, 128), 128)
            g_s[f * 128:(f + 1) * 128, :] = bqkv_st[r, c].astype(F32).T
        for t in range(NT):
            c = pl.ds(pl.multiple_of(j * D + t * 128, 128), 128)
            bqkv_s[pl.ds(pl.multiple_of(a * 64, 64), 64), c] = _pack(gather_heads(t).T.astype(BF16))

    def perm_wo():
        for f in range(NT):
            c = slice(f * 128, (f + 1) * 128)
            g_s[...] = bwo_st[:, c].astype(F32)
            for t in range(NT):
                bwo_s[t * 64:(t + 1) * 64, c] = _pack(gather_heads(t).astype(BF16))

    def b_ln(seg):
        hbbuf[...] = _layernorm(xs[rows(seg), :])

    def b_proj(seg, j):
        y = _dot(hbbuf[...], _unpack(bqkv_s[:, j * D:(j + 1) * D]))
        if j == 0:
            qbuf[...] = y * b_scale
        else:
            buf = kbuf if j == 1 else vbuf
            buf[0:TAIL, :] = jnp.where(seg == 0, 0.0, buf[SEG:SEG + TAIL, :])
            buf[TAIL:, :] = y

    def b_logit(st, seg, w):
        off = TAIL - DIL * w
        s = None
        for j in range(NT):
            c = slice(j * 128, (j + 1) * 128)
            t = qbuf[:, c] * kbuf[off:off + SEG, c]
            s = t if s is None else s + t
        s = s + pltpu.roll(s, 64, 1)
        s = s + pltpu.roll(s, 32, 1)
        if w > 0:
            pos = lax.broadcasted_iota(jnp.int32, (SEG, 128), 0) + seg * SEG
            s = jnp.where(pos >= DIL * w, s, NEG)
        st.setdefault("blog", []).append(s)

    def b_softmax(st):
        logits = st["blog"]
        m = functools.reduce(jnp.maximum, logits)
        st["bexp"] = [jnp.exp(s - m) for s in logits]
        st["binv"] = _recip(functools.reduce(jnp.add, st["bexp"]))

    def b_pv(st, j):
        c = slice(j * 128, (j + 1) * 128)
        oj = None
        for w in range(W):
            off = TAIL - DIL * w
            t = st["bexp"][w] * vbuf[off:off + SEG, c]
            oj = t if oj is None else oj + t
        st.setdefault("bo", []).append(oj * st["binv"])

    def b_out(st, seg, active):
        x1 = xs[rows(seg), :]
        x2 = x1 + _dot(jnp.concatenate(st["bo"], axis=1), _unpack(bwo_s[...]))
        x2 = jnp.where(active, x2, x1)
        xs[rows(seg), :] = x2
        out_st[rows(seg), :] = x2.astype(out_st.dtype)

    def a_proj(st, p, j):
        y = _dot(st["h"], _unpack(w_s[p, :, j * PW:(j + 1) * PW]))
        if "pre" in st:
            y = jnp.concatenate([y, pre_s[p, st["pre"], j * PW:(j + 1) * PW]], axis=0)
        st["qkv"[j], p] = y

    def split_heads(t):
        lo = lax.broadcasted_iota(jnp.int32, (L, 128), 1) < (DH - 128)
        z = jnp.zeros((L, 128), F32)
        t0, t1, t2 = t[:, 0:128], t[:, 128:256], t[:, 256:384]
        top = jnp.concatenate([t0, jnp.where(lo, t1, 0.0), z], axis=1)
        bot = jnp.concatenate([z, jnp.where(lo, 0.0, t1), t2], axis=1)
        return jnp.concatenate([top, bot], axis=0).astype(BF16)

    def score_masks():
        row = lax.broadcasted_iota(jnp.int32, (L, 128), 0)
        col = lax.broadcasted_iota(jnp.int32, (L, 128), 1)
        lo = col < L
        key = jnp.where(lo, col, col - L)
        visible = ((row < M) | (row >= key)) & (col < 2 * L)
        fill = jnp.where(col < 2 * L, NEG, -jnp.inf)
        return lo, visible, fill

    def a_qk(st, p):
        st["s", p] = _dot_nt(st["q", p], split_heads(st["k", p]))

    def a_max(st, p):
        lo, visible, fill = score_masks()
        s = jnp.concatenate([st["s", p], jnp.zeros((L, 128 - 2 * L), F32)], axis=1)
        s = jnp.where(visible, s * a_scale, fill)
        m_lo = jnp.max(jnp.where(lo, s, -jnp.inf), axis=-1, keepdims=True)
        m_hi = jnp.max(jnp.where(lo, -jnp.inf, s), axis=-1, keepdims=True)
        st["s", p] = s
        st["m", p] = (m_lo, m_hi)

    def a_exp(st, p):
        lo = score_masks()[0]
        m_lo, m_hi = st["m", p]
        e = jnp.exp(st["s", p] - jnp.where(lo, m_lo, m_hi))
        d_lo = jnp.sum(jnp.where(lo, e, 0.0), axis=-1, keepdims=True)
        d_hi = jnp.sum(jnp.where(lo, 0.0, e), axis=-1, keepdims=True)
        st["e", p] = e
        st["d", p] = (d_lo, d_hi)

    def a_norm(st, p):
        lo = score_masks()[0]
        d_lo, d_hi = st["d", p]
        vb = jnp.concatenate([split_heads(st["v", p]), jnp.zeros((128 - 2 * L, PW), BF16)], axis=0)
        return st["e", p] * _recip(jnp.where(lo, d_lo, d_hi)), vb

    def a_pv(st, p):
        st["o", p] = _dot(*a_norm(st, p))

    def a_out(st, p):
        y = _dot(st["o", p], _unpack(wo_s[p]))
        st["acc"] = y if "acc" not in st else st["acc"] + y

    cp_x0.start()
    cp_xp.start()
    cp_q0.start()

    kbuf[...] = jnp.zeros(kbuf.shape, F32)
    vbuf[...] = jnp.zeros(vbuf.shape, F32)
    qbuf[...] = jnp.zeros(qbuf.shape, F32)
    hbbuf[...] = jnp.zeros(hbbuf.shape, F32)
    mem0 = mem0_ref[...].astype(F32)

    def load_x(lo, hi):
        for i in range(lo, hi):
            xs[i * SEG:(i + 1) * SEG, :] = x_st[i].astype(F32)

    cp_k0.start()
    cp_x0.wait()
    load_x(0, 2)
    cp_xp.wait()
    cp_v0.start()
    hall_s[0:M, :] = mem0
    hall_s[M:L, :] = _layernorm(xs[0:SEG, :])
    hall_s[L:, :] = _layernorm(xp_st[...].astype(F32).reshape(NPRE * PR, D))

    def start_pair(p):
        for cp in wcopies(p):
            cp.start()
        bcopy(p).start()

    def first_pair(p, carry, head=False):
        acc, pr_prev, vb_prev = carry
        r = pl.ds(pl.multiple_of(p * PW, PW), PW)
        st = {}

        def proj(j):
            y = _dot_nt(hall_s[...], (q_st, k_st, v_st)[j][r, :])
            st["qkv"[j], 0] = y[:L, :]
            pre_s[p, :, j * PW:(j + 1) * PW] = y[L:, :]

        def repack(j):
            w_s[p, :, j * PW:(j + 1) * PW] = _pack((q_st, k_st, v_st)[j][r, :].T)

        if head:
            cp_q0.wait()
            cp_o0.start()
            bcopy(0).start()
            cp_x0b.start()
            proj(0)
            repack(0)
            cp_k0.wait()
            start_pair(1)
            proj(1)
            a_qk(st, 0)
            repack(1)
            cp_v0.wait()
            start_pair(2)
            proj(2)
            a_max(st, 0)
            a_exp(st, 0)
            repack(2)
            cp_o0.wait()
            bcopy(0).wait()
            perm_wqkv_piece(0)
            wo_s[p] = _pack(o_st[r, :])
            return (acc,) + a_norm(st, 0)

        for cp in wcopies(p):
            cp.wait()

        @pl.when(p < NU)
        def _():
            bcopy(jnp.minimum(p, NU - 1)).wait()

        @pl.when(p + 2 < NP)
        def _():
            for cp in wcopies(jnp.minimum(p + 2, NP - 1)):
                cp.start()

        @pl.when(p + 2 < NU)
        def _():
            bcopy(jnp.minimum(p + 2, NU - 1)).start()

        @pl.when(p + 2 == NP)
        def _():
            cp_bo.start()
            cp_x1.start()

        rprev = pl.ds(pl.multiple_of(jnp.maximum(p - 1, 0) * PW, PW), PW)
        proj(0)
        o_prev = _dot(pr_prev, vb_prev)
        proj(1)
        acc = acc + _dot(o_prev, o_st[rprev, :])
        a_qk(st, 0)
        repack(0)
        proj(2)
        a_max(st, 0)
        perm_wqkv_piece(jnp.minimum(p, NU - 1))
        repack(1)
        a_exp(st, 0)
        repack(2)
        wo_s[p] = _pack(o_st[r, :])
        return (acc,) + a_norm(st, 0)

    carry = first_pair(0, (jnp.zeros((L, D), F32), None, None), head=True)
    acc0, pr, vb = lax.fori_loop(1, NP, first_pair, carry)
    cp_x0b.wait()
    load_x(2, X0)
    cp_bo.wait()
    acc0 = acc0 + _dot(_dot(pr, vb), o_st[(NP - 1) * PW:NP * PW, :])
    perm_wo()
    xs[0:SEG, :] = xs[0:SEG, :] + acc0[M:, :]
    hbuf[...] = _layernorm(xs[SEG:2 * SEG, :])

    GX = X0 - 1 - (X0 - 2) % UNROLL
    assert NPRE % UNROLL == 0 and (NG - 2 - NPRE) % UNROLL == 0 and X0 <= NPRE < NSEG
    assert X0 + 2 * (NPRE - GX) + 1 >= NSEG - 1
    schedule = _schedule(NP, W, NT)

    def step(g, mem, pre=False):
        seg = g % NSEG
        seg1 = (g + NSEG - 1) % NSEG
        seg2 = jnp.maximum(g - 2, 0) % NSEG
        segn = (g + 1) % NSEG
        mem = jnp.where(seg == 0, mem0, mem)
        first_out = NSEG + OC // SEG + 2

        @pl.when((g >= first_out) & ((g - first_out) % (OC // SEG) == 0))
        def _():
            lo = pl.multiple_of((g - first_out) // (OC // SEG) * OC, OC)
            ocopy_dyn(lo).start()

        if pre:
            st = {"h": jnp.concatenate([mem, hbuf[0:SEG - PR, :]], axis=0),
                  "pre": pl.ds(pl.multiple_of((g - 1) * PR, PR), PR)}
        else:
            st = {"h": jnp.concatenate([mem, hbuf[...]], axis=0)}

        for op, *arg in schedule:
            if op in ("q", "k", "v"):
                a_proj(st, arg[0], "qkv".index(op))
            elif op == "qk":
                a_qk(st, arg[0])
            elif op == "max":
                a_max(st, arg[0])
            elif op == "exp":
                a_exp(st, arg[0])
            elif op == "pv":
                a_pv(st, arg[0])
            elif op == "out":
                a_out(st, arg[0])
            elif op == "blog":
                b_logit(st, seg2, arg[0])
            elif op == "bsm":
                b_softmax(st)
            elif op == "bpv":
                b_pv(st, arg[0])
            elif op == "bout":
                b_out(st, seg2, g >= 2)
            elif op == "bln":
                b_ln(seg1)
            elif op == "bproj":
                b_proj(seg1, arg[0])
            elif op == "xupd":
                xs[rows(seg), :] = xs[rows(seg), :] + st["acc"][M:, :]
            elif op == "xcvt":
                if pre:
                    for u in range(2):
                        c = jnp.where(g >= GX, jnp.minimum(X0 + 2 * (g - GX) + u, NSEG - 1), X0 - 1)
                        xs[rows(c), :] = x_st[c].astype(F32)
            elif op == "hln":
                hbuf[...] = _layernorm(xs[rows(segn), :])
            else:
                raise ValueError(op)
        return st["acc"][:M, :]

    def ocopy_dyn(lo):
        r = pl.ds(lo, OC)
        return pltpu.make_async_copy(out_st.at[r, :], out_hbm.at[r, :], osem.at[0])

    def body_pre(i, mem):
        @pl.when(i == GX // UNROLL)
        def _():
            cp_x1.wait()
        for u in range(UNROLL):
            mem = step(1 + i * UNROLL + u, mem, pre=True)
        return mem

    def body(i, mem):
        for u in range(UNROLL):
            mem = step(1 + NPRE + i * UNROLL + u, mem)
        return mem

    mem = lax.fori_loop(0, NPRE // UNROLL, body_pre, acc0[:M, :])
    mem = lax.fori_loop(0, (NG - 2 - NPRE) // UNROLL, body, mem)
    step(NG - 1, mem)

    last = S - 2 * SEG
    cp_last = [ocopy(S - OC, last), ocopy(last, S)]
    cp_last[0].start()
    for seg in (NSEG - 2, NSEG - 1):
        st = {}
        for w in range(W):
            b_logit(st, seg, w)
        b_softmax(st)
        for j in range(NT):
            b_pv(st, j)
        if seg == NSEG - 2:
            b_ln(NSEG - 1)
        b_out(st, seg, True)
        if seg == NSEG - 2:
            for j in range(3):
                b_proj(NSEG - 1, j)
    cp_last[1].start()
    for c in range(NOC - 1):
        ocopy(c * OC, (c + 1) * OC).wait()
    for cp in cp_last:
        cp.wait()


@functools.partial(jax.jit, static_argnames=("A_seg_len",))
def pallas_interleave_layers__memory_aug_recurrent_mem_tr__sliding_local_dilated__prompt_kernel(
    A_x, A_mem0, A_Wq, A_Wk, A_Wv, A_Wo, A_seg_len, B_x, B_wqkv, B_wo,
):
    del B_x
    B, S, D = A_x.shape
    M = A_mem0.shape[1]
    _, H, DH = A_Wq.shape
    SEG = int(A_seg_len)
    HB, W, DIL = 32, 8, 2
    assert B == 1 and S % 256 == 0 and H % 2 == 0 and 2 * DH == 384 and D % 128 == 0

    def wt(w):
        return w.transpose(1, 2, 0).reshape(H * DH, D)

    hbm = pl.BlockSpec(memory_space=pl.ANY)
    out = pl.pallas_call(
        functools.partial(_kernel, S=S, D=D, H=H, DH=DH, M=M, SEG=SEG, W=W, DIL=DIL, HB=HB),
        out_shape=jax.ShapeDtypeStruct((S, D), A_x.dtype),
        in_specs=[hbm, pl.BlockSpec(memory_space=pltpu.VMEM), hbm, hbm, hbm, hbm, hbm, hbm],
        out_specs=hbm,
        scratch_shapes=[
            pltpu.VMEM((S, D), F32),
            pltpu.VMEM((H // 2, D // 2, 6 * DH), U32),
            pltpu.VMEM((H // 2, DH, D), U32),
            pltpu.VMEM((D // 2, 3 * D), U32),
            pltpu.VMEM((D // 2, D), U32),
            pltpu.VMEM((SEG, D), F32),
            pltpu.VMEM((SEG, D), F32),
            pltpu.VMEM((SEG, D), F32),
            pltpu.VMEM((16 + SEG, D), F32),
            pltpu.VMEM((16 + SEG, D), F32),
            pltpu.VMEM((S // SEG, SEG, D), BF16),
            pltpu.VMEM((H * DH, D), BF16),
            pltpu.VMEM((H * DH, D), BF16),
            pltpu.VMEM((H * DH, D), BF16),
            pltpu.VMEM((H * DH, D), BF16),
            pltpu.VMEM((D, 3 * D), BF16),
            pltpu.VMEM((D, D), BF16),
            pltpu.VMEM((S, D), BF16),
            pltpu.VMEM((D, 128), F32),
            pltpu.VMEM((NPRE, PR, D), BF16),
            pltpu.VMEM((M + SEG + NPRE * PR, D), F32),
            pltpu.VMEM((H // 2, NPRE * PR, 6 * DH), F32),
            pltpu.SemaphoreType.DMA((4, H // 2)),
            pltpu.SemaphoreType.DMA((3 * D // 128,)),
            pltpu.SemaphoreType.DMA((5,)),
            pltpu.SemaphoreType.DMA((1,)),
        ],
        compiler_params=pltpu.CompilerParams(vmem_limit_bytes=120 * 1024 * 1024),
    )(A_x.reshape(S // SEG, SEG, D), A_mem0.reshape(M, D), wt(A_Wq), wt(A_Wk), wt(A_Wv),
      A_Wo.reshape(H * DH, D), B_wqkv, B_wo)
    return out.reshape(B, S, D)
```

```python
import functools

import jax
import jax.numpy as jnp
import numpy as np
from jax import lax
from jax.experimental import pallas as pl
from jax.experimental.pallas import tpu as pltpu

F32 = jnp.float32
BF16 = jnp.bfloat16
U32 = jnp.uint32
NEG = -1000000000.0

NPRE = 36
PR = 8
UNROLL = 2


def _bf16_const(v):
    return float(np.asarray(v, dtype=BF16).astype(np.float32))


def _dot(a, b):
    return lax.dot_general(a, b, (((1,), (0,)), ((), ())), preferred_element_type=F32)


def _dot_nt(a, b):
    return lax.dot_general(a, b, (((1,), (1,)), ((), ())), preferred_element_type=F32)


def _layernorm(x):
    m = jnp.mean(x, axis=-1, keepdims=True)
    c = x - m
    v = jnp.mean(c * c, axis=-1, keepdims=True)
    return c * lax.rsqrt(v + 1e-5)


def _pack(x):
    return pltpu.bitcast(x, U32)


def _unpack(x):
    return pltpu.bitcast(x, BF16)


def _recip(d):
    r = pl.reciprocal(d, approx=True)
    return r * (2.0 - d * r)


ORDER_PRE = (
    "k0 q0 v0 q1 s0 k1 v1 q2 s1 p0 k2 q3 v2 s2 p1 k3 v3 q4 s3 p2 k4 v4 q5 s4 p3 k5 v5 q6 s5 "
    "p4 k6 v6 q7 s6 p5 k7 o0 v7 q8 s7 p6 k8 v8 o1 B q9 s8 p7 v9 k9 o2 q10 s9 p8 k10 o3 v10 "
    "q11 s10 p9 k11 v11 o4 q12 s11 p10 k12 v12 o5 q13 s12 p11 k13 v13 o6 q14 s13 p12 v14 k14 "
    "o7 q15 s14 p13 k15 v15 o8 s15 p14 o9 o10 o11 o13 p15 o12 o14 o15 b2 b0 b1 ")
ORDER_MAIN = (
    "q0 k0 v0 q1 s0 k1 v1 q2 s1 k2 v2 v3 p0 q3 s2 k3 p1 q4 s3 k4 v4 p2 q5 k5 v5 s4 q6 p3 s5 "
    "k6 v6 p4 q7 s6 o0 k7 v7 o1 p5 q8 s7 k8 v8 p6 B o2 q9 s8 k9 v9 q10 s9 p7 o3 k10 p8 v10 "
    "q11 s10 o4 k11 p9 v11 q12 s11 o5 k12 v12 q13 p10 s12 v13 k13 o6 p11 q14 s13 k14 o7 v14 "
    "p12 q15 s14 o8 k15 v15 p13 s15 p14 o10 o9 o11 o13 o14 o12 p15 b0 o15 b1 b2 ")


def _schedule(order, n_window, n_tiles):
    names = {"q": "q", "k": "k", "v": "v", "s": "qk", "p": "pv", "o": "out", "B": "bout", "b": "bproj"}
    mm = [(names[t[0]],) + ((int(t[1:]),) if t[1:] else ()) for t in order.split()]
    bwork = ([("blog", w) for w in range(n_window)] + [("bsm",)]
             + [("bpv", j) for j in range(n_tiles)])
    every = max(1, mm.index(("bout",)) // len(bwork))
    last_out = max(i for i, op in enumerate(mm) if op[0] == "out")
    s = []
    for i, op in enumerate(mm):
        if op == ("bout",):
            s += bwork
            bwork = []
        s.append(op)
        if op[0] == "qk":
            s += [("max", op[1]), ("exp", op[1])]
        if bwork and i % every == every - 1:
            s.append(bwork.pop(0))
        if op == ("bout",):
            s += [("xcvt",), ("bln",), ("hln",)]
        if i == last_out:
            s.append(("xupd",))
    return s


def _kernel(x_hbm, mem0_ref, wqt_hbm, wkt_hbm, wvt_hbm, wo_hbm, bqkv_hbm, bwo_hbm,
            out_hbm,
            xs, w_s, wo_s, bqkv_s, bwo_s, hbuf, hbbuf, qbuf, kbuf, vbuf,
            x_st, q_st, k_st, v_st, o_st, bqkv_st, bwo_st, out_st, g_s, xp_st, hall_s, pre_s,
            wsem, bsem, msem, osem,
            *, S, D, H, DH, M, SEG, W, DIL, HB):
    NSEG = S // SEG
    NG = 2 * NSEG
    L = M + SEG
    NP = H // 2
    PW = 2 * DH
    NT = D // 128
    DB = D // HB
    NU = 3 * NT
    TAIL = 16
    OC = 256
    NOC = S // OC
    X0 = 256 // SEG
    a_scale = _bf16_const(DH ** -0.5)
    b_scale = _bf16_const(DB ** -0.5)
    assert DIL * (W - 1) <= TAIL and 128 % HB == 0 and NU <= NP - 1

    def wcopies(p):
        r = pl.ds(p * PW, PW)
        return [pltpu.make_async_copy(src.at[r, :], dst.at[r, :], wsem.at[i, p])
                for i, (src, dst) in enumerate(
                    ((wqt_hbm, q_st), (wkt_hbm, k_st), (wvt_hbm, v_st), (wo_hbm, o_st)))]

    def bcopy(u):
        r = pl.ds(pl.multiple_of((u % NT) * 128, 128), 128)
        c = pl.ds(pl.multiple_of((u // NT) * D, 128), D)
        return pltpu.make_async_copy(bqkv_hbm.at[r, c], bqkv_st.at[r, c], bsem.at[u])

    def ocopy(lo, hi):
        return pltpu.make_async_copy(out_st.at[pl.ds(lo, hi - lo), :],
                                     out_hbm.at[pl.ds(lo, hi - lo), :], osem.at[0])

    cp_x0 = pltpu.make_async_copy(x_hbm.at[0:2], x_st.at[0:2], msem.at[0])
    cp_x0b = pltpu.make_async_copy(x_hbm.at[2:X0], x_st.at[2:X0], msem.at[1])
    cp_x1 = pltpu.make_async_copy(x_hbm.at[X0:NSEG], x_st.at[X0:NSEG], msem.at[2])
    cp_xp = pltpu.make_async_copy(x_hbm.at[1:NPRE + 1, SEG - PR:SEG, :], xp_st, msem.at[3])
    cp_bo = pltpu.make_async_copy(bwo_hbm, bwo_st, msem.at[4])
    cp_q0, cp_k0, cp_v0, cp_o0 = wcopies(0)

    def rows(seg):
        return pl.ds(pl.multiple_of(seg * SEG, SEG), SEG)

    def gather_heads(t):
        n = 128 // HB
        return jnp.concatenate(
            [g_s[pl.ds(n * t + dd, HB, stride=DB), :] for dd in range(n)], axis=0)

    def perm_wqkv_piece(u):
        j, a = u // NT, u % NT
        r = pl.ds(pl.multiple_of(a * 128, 128), 128)
        for f in range(NT):
            c = pl.ds(pl.multiple_of(j * D + f * 128, 128), 128)
            g_s[f * 128:(f + 1) * 128, :] = bqkv_st[r, c].astype(F32).T
        for t in range(NT):
            c = pl.ds(pl.multiple_of(j * D + t * 128, 128), 128)
            bqkv_s[pl.ds(pl.multiple_of(a * 64, 64), 64), c] = _pack(gather_heads(t).T.astype(BF16))

    def perm_wo():
        for f in range(NT):
            c = slice(f * 128, (f + 1) * 128)
            g_s[...] = bwo_st[:, c].astype(F32)
            for t in range(NT):
                bwo_s[t * 64:(t + 1) * 64, c] = _pack(gather_heads(t).astype(BF16))

    def b_ln(seg):
        hbbuf[...] = _layernorm(xs[rows(seg), :])

    def b_proj(seg, j):
        y = _dot(hbbuf[...], _unpack(bqkv_s[:, j * D:(j + 1) * D]))
        if j == 0:
            qbuf[...] = y * b_scale
        else:
            buf = kbuf if j == 1 else vbuf
            buf[0:TAIL, :] = jnp.where(seg == 0, 0.0, buf[SEG:SEG + TAIL, :])
            buf[TAIL:, :] = y

    def b_logit(st, seg, w):
        off = TAIL - DIL * w
        s = None
        for j in range(NT):
            c = slice(j * 128, (j + 1) * 128)
            t = qbuf[:, c] * kbuf[off:off + SEG, c]
            s = t if s is None else s + t
        s = s + pltpu.roll(s, 64, 1)
        s = s + pltpu.roll(s, 32, 1)
        if w > 0:
            pos = lax.broadcasted_iota(jnp.int32, (SEG, 128), 0) + seg * SEG
            s = jnp.where(pos >= DIL * w, s, NEG)
        st.setdefault("blog", []).append(s)

    def b_softmax(st):
        logits = st["blog"]
        m = functools.reduce(jnp.maximum, logits)
        st["bexp"] = [jnp.exp(s - m) for s in logits]
        st["binv"] = _recip(functools.reduce(jnp.add, st["bexp"]))

    def b_pv(st, j):
        c = slice(j * 128, (j + 1) * 128)
        oj = None
        for w in range(W):
            off = TAIL - DIL * w
            t = st["bexp"][w] * vbuf[off:off + SEG, c]
            oj = t if oj is None else oj + t
        st.setdefault("bo", []).append(oj * st["binv"])

    def b_out(st, seg, active):
        x1 = xs[rows(seg), :]
        x2 = x1 + _dot(jnp.concatenate(st["bo"], axis=1), _unpack(bwo_s[...]))
        x2 = jnp.where(active, x2, x1)
        xs[rows(seg), :] = x2
        out_st[rows(seg), :] = x2.astype(out_st.dtype)

    def a_proj(st, p, j):
        y = _dot(st["h"], _unpack(w_s[p, :, j * PW:(j + 1) * PW]))
        if "pre" in st:
            y = jnp.concatenate([y, pre_s[p, st["pre"], j * PW:(j + 1) * PW]], axis=0)
        st["qkv"[j], p] = y

    def split_heads(t):
        lo = lax.broadcasted_iota(jnp.int32, (L, 128), 1) < (DH - 128)
        z = jnp.zeros((L, 128), F32)
        t0, t1, t2 = t[:, 0:128], t[:, 128:256], t[:, 256:384]
        top = jnp.concatenate([t0, jnp.where(lo, t1, 0.0), z], axis=1)
        bot = jnp.concatenate([z, jnp.where(lo, 0.0, t1), t2], axis=1)
        return jnp.concatenate([top, bot], axis=0).astype(BF16)

    def score_masks():
        row = lax.broadcasted_iota(jnp.int32, (L, 128), 0)
        col = lax.broadcasted_iota(jnp.int32, (L, 128), 1)
        lo = col < L
        key = jnp.where(lo, col, col - L)
        visible = ((row < M) | (row >= key)) & (col < 2 * L)
        fill = jnp.where(col < 2 * L, NEG, -jnp.inf)
        return lo, visible, fill

    def a_qk(st, p):
        st["s", p] = _dot_nt(st["q", p], split_heads(st["k", p]))

    def a_max(st, p):
        lo, visible, fill = score_masks()
        s = jnp.concatenate([st["s", p], jnp.zeros((L, 128 - 2 * L), F32)], axis=1)
        s = jnp.where(visible, s * a_scale, fill)
        m_lo = jnp.max(jnp.where(lo, s, -jnp.inf), axis=-1, keepdims=True)
        m_hi = jnp.max(jnp.where(lo, -jnp.inf, s), axis=-1, keepdims=True)
        st["s", p] = s
        st["m", p] = (m_lo, m_hi)

    def a_exp(st, p):
        lo = score_masks()[0]
        m_lo, m_hi = st["m", p]
        e = jnp.exp(st["s", p] - jnp.where(lo, m_lo, m_hi))
        d_lo = jnp.sum(jnp.where(lo, e, 0.0), axis=-1, keepdims=True)
        d_hi = jnp.sum(jnp.where(lo, 0.0, e), axis=-1, keepdims=True)
        st["e", p] = e
        st["d", p] = (d_lo, d_hi)

    def a_norm(st, p):
        lo = score_masks()[0]
        d_lo, d_hi = st["d", p]
        vb = jnp.concatenate([split_heads(st["v", p]), jnp.zeros((128 - 2 * L, PW), BF16)], axis=0)
        return st["e", p] * _recip(jnp.where(lo, d_lo, d_hi)), vb

    def a_pv(st, p):
        st["o", p] = _dot(*a_norm(st, p))

    def a_out(st, p):
        y = _dot(st["o", p], _unpack(wo_s[p]))
        st["acc"] = y if "acc" not in st else st["acc"] + y

    cp_x0.start()
    cp_xp.start()
    cp_q0.start()

    kbuf[...] = jnp.zeros(kbuf.shape, F32)
    vbuf[...] = jnp.zeros(vbuf.shape, F32)
    qbuf[...] = jnp.zeros(qbuf.shape, F32)
    hbbuf[...] = jnp.zeros(hbbuf.shape, F32)
    mem0 = mem0_ref[...].astype(F32)

    def load_x(lo, hi):
        for i in range(lo, hi):
            xs[i * SEG:(i + 1) * SEG, :] = x_st[i].astype(F32)

    cp_k0.start()
    cp_x0.wait()
    load_x(0, 2)
    cp_xp.wait()
    cp_v0.start()
    hall_s[0:M, :] = mem0
    hall_s[M:L, :] = _layernorm(xs[0:SEG, :])
    hall_s[L:, :] = _layernorm(xp_st[...].astype(F32).reshape(NPRE * PR, D))

    def start_pair(p):
        for cp in wcopies(p):
            cp.start()
        bcopy(p).start()

    def first_pair(p, carry, head=False):
        acc, pr_prev, vb_prev = carry
        r = pl.ds(pl.multiple_of(p * PW, PW), PW)
        st = {}

        def proj(j):
            y = _dot_nt(hall_s[...], (q_st, k_st, v_st)[j][r, :])
            st["qkv"[j], 0] = y[:L, :]
            pre_s[p, :, j * PW:(j + 1) * PW] = y[L:, :]

        def repack(j):
            w_s[p, :, j * PW:(j + 1) * PW] = _pack((q_st, k_st, v_st)[j][r, :].T)

        if head:
            cp_q0.wait()
            cp_o0.start()
            bcopy(0).start()
            cp_x0b.start()
            proj(0)
            repack(0)
            cp_k0.wait()
            start_pair(1)
            proj(1)
            a_qk(st, 0)
            repack(1)
            cp_v0.wait()
            start_pair(2)
            proj(2)
            a_max(st, 0)
            a_exp(st, 0)
            repack(2)
            cp_o0.wait()
            bcopy(0).wait()
            perm_wqkv_piece(0)
            wo_s[p] = _pack(o_st[r, :])
            return (acc,) + a_norm(st, 0)

        for cp in wcopies(p):
            cp.wait()

        @pl.when(p < NU)
        def _():
            bcopy(jnp.minimum(p, NU - 1)).wait()

        @pl.when(p + 2 < NP)
        def _():
            for cp in wcopies(jnp.minimum(p + 2, NP - 1)):
                cp.start()

        @pl.when(p + 2 < NU)
        def _():
            bcopy(jnp.minimum(p + 2, NU - 1)).start()

        @pl.when(p + 2 == NP)
        def _():
            cp_bo.start()
            cp_x1.start()

        rprev = pl.ds(pl.multiple_of(jnp.maximum(p - 1, 0) * PW, PW), PW)
        proj(0)
        o_prev = _dot(pr_prev, vb_prev)
        proj(1)
        acc = acc + _dot(o_prev, o_st[rprev, :])
        a_qk(st, 0)
        repack(0)
        proj(2)
        a_max(st, 0)
        perm_wqkv_piece(jnp.minimum(p, NU - 1))
        repack(1)
        a_exp(st, 0)
        repack(2)
        wo_s[p] = _pack(o_st[r, :])
        return (acc,) + a_norm(st, 0)

    carry = first_pair(0, (jnp.zeros((L, D), F32), None, None), head=True)
    acc0, pr, vb = lax.fori_loop(1, NP, first_pair, carry)
    cp_x0b.wait()
    load_x(2, X0)
    cp_bo.wait()
    acc0 = acc0 + _dot(_dot(pr, vb), o_st[(NP - 1) * PW:NP * PW, :])
    perm_wo()
    xs[0:SEG, :] = xs[0:SEG, :] + acc0[M:, :]
    hbuf[...] = _layernorm(xs[SEG:2 * SEG, :])

    GX = X0 - 1 - (X0 - 2) % UNROLL
    assert NPRE % UNROLL == 0 and (NG - 2 - NPRE) % UNROLL == 0 and X0 <= NPRE < NSEG
    assert X0 + 2 * (NPRE - GX) + 1 >= NSEG - 1
    assert NP == 16
    schedules = {True: _schedule(ORDER_PRE, W, NT), False: _schedule(ORDER_MAIN, W, NT)}

    def step(g, mem, pre=False):
        seg = g % NSEG
        seg1 = (g + NSEG - 1) % NSEG
        seg2 = jnp.maximum(g - 2, 0) % NSEG
        segn = (g + 1) % NSEG
        mem = jnp.where(seg == 0, mem0, mem)
        first_out = NSEG + OC // SEG + 2

        @pl.when((g >= first_out) & ((g - first_out) % (OC // SEG) == 0))
        def _():
            lo = pl.multiple_of((g - first_out) // (OC // SEG) * OC, OC)
            ocopy_dyn(lo).start()

        if pre:
            st = {"h": jnp.concatenate([mem, hbuf[0:SEG - PR, :]], axis=0),
                  "pre": pl.ds(pl.multiple_of((g - 1) * PR, PR), PR)}
        else:
            st = {"h": jnp.concatenate([mem, hbuf[...]], axis=0)}

        for op, *arg in schedules[pre]:
            if op in ("q", "k", "v"):
                a_proj(st, arg[0], "qkv".index(op))
            elif op == "qk":
                a_qk(st, arg[0])
            elif op == "max":
                a_max(st, arg[0])
            elif op == "exp":
                a_exp(st, arg[0])
            elif op == "pv":
                a_pv(st, arg[0])
            elif op == "out":
                a_out(st, arg[0])
            elif op == "blog":
                b_logit(st, seg2, arg[0])
            elif op == "bsm":
                b_softmax(st)
            elif op == "bpv":
                b_pv(st, arg[0])
            elif op == "bout":
                b_out(st, seg2, g >= 2)
            elif op == "bln":
                b_ln(seg1)
            elif op == "bproj":
                b_proj(seg1, arg[0])
            elif op == "xupd":
                xs[rows(seg), :] = xs[rows(seg), :] + st["acc"][M:, :]
            elif op == "xcvt":
                if pre:
                    for u in range(2):
                        c = jnp.where(g >= GX, jnp.minimum(X0 + 2 * (g - GX) + u, NSEG - 1), X0 - 1)
                        xs[rows(c), :] = x_st[c].astype(F32)
            elif op == "hln":
                hbuf[...] = _layernorm(xs[rows(segn), :])
            else:
                raise ValueError(op)
        return st["acc"][:M, :]

    def ocopy_dyn(lo):
        r = pl.ds(lo, OC)
        return pltpu.make_async_copy(out_st.at[r, :], out_hbm.at[r, :], osem.at[0])

    def body_pre(i, mem):
        @pl.when(i == GX // UNROLL)
        def _():
            cp_x1.wait()
        for u in range(UNROLL):
            mem = step(1 + i * UNROLL + u, mem, pre=True)
        return mem

    def body(i, mem):
        for u in range(UNROLL):
            mem = step(1 + NPRE + i * UNROLL + u, mem)
        return mem

    mem = lax.fori_loop(0, NPRE // UNROLL, body_pre, acc0[:M, :])
    mem = lax.fori_loop(0, (NG - 2 - NPRE) // UNROLL, body, mem)
    step(NG - 1, mem)

    last = S - 2 * SEG
    cp_last = [ocopy(S - OC, last), ocopy(last, S)]
    cp_last[0].start()
    for seg in (NSEG - 2, NSEG - 1):
        st = {}
        for w in range(W):
            b_logit(st, seg, w)
        b_softmax(st)
        for j in range(NT):
            b_pv(st, j)
        if seg == NSEG - 2:
            b_ln(NSEG - 1)
        b_out(st, seg, True)
        if seg == NSEG - 2:
            for j in range(3):
                b_proj(NSEG - 1, j)
    cp_last[1].start()
    for c in range(NOC - 1):
        ocopy(c * OC, (c + 1) * OC).wait()
    for cp in cp_last:
        cp.wait()


@functools.partial(jax.jit, static_argnames=("A_seg_len",))
def pallas_interleave_layers__memory_aug_recurrent_mem_tr__sliding_local_dilated__prompt_kernel(
    A_x, A_mem0, A_Wq, A_Wk, A_Wv, A_Wo, A_seg_len, B_x, B_wqkv, B_wo,
):
    del B_x
    B, S, D = A_x.shape
    M = A_mem0.shape[1]
    _, H, DH = A_Wq.shape
    SEG = int(A_seg_len)
    HB, W, DIL = 32, 8, 2
    assert B == 1 and S % 256 == 0 and H % 2 == 0 and 2 * DH == 384 and D % 128 == 0

    def wt(w):
        return w.transpose(1, 2, 0).reshape(H * DH, D)

    hbm = pl.BlockSpec(memory_space=pl.ANY)
    out = pl.pallas_call(
        functools.partial(_kernel, S=S, D=D, H=H, DH=DH, M=M, SEG=SEG, W=W, DIL=DIL, HB=HB),
        out_shape=jax.ShapeDtypeStruct((S, D), A_x.dtype),
        in_specs=[hbm, pl.BlockSpec(memory_space=pltpu.VMEM), hbm, hbm, hbm, hbm, hbm, hbm],
        out_specs=hbm,
        scratch_shapes=[
            pltpu.VMEM((S, D), F32),
            pltpu.VMEM((H // 2, D // 2, 6 * DH), U32),
            pltpu.VMEM((H // 2, DH, D), U32),
            pltpu.VMEM((D // 2, 3 * D), U32),
            pltpu.VMEM((D // 2, D), U32),
            pltpu.VMEM((SEG, D), F32),
            pltpu.VMEM((SEG, D), F32),
            pltpu.VMEM((SEG, D), F32),
            pltpu.VMEM((16 + SEG, D), F32),
            pltpu.VMEM((16 + SEG, D), F32),
            pltpu.VMEM((S // SEG, SEG, D), BF16),
            pltpu.VMEM((H * DH, D), BF16),
            pltpu.VMEM((H * DH, D), BF16),
            pltpu.VMEM((H * DH, D), BF16),
            pltpu.VMEM((H * DH, D), BF16),
            pltpu.VMEM((D, 3 * D), BF16),
            pltpu.VMEM((D, D), BF16),
            pltpu.VMEM((S, D), BF16),
            pltpu.VMEM((D, 128), F32),
            pltpu.VMEM((NPRE, PR, D), BF16),
            pltpu.VMEM((M + SEG + NPRE * PR, D), F32),
            pltpu.VMEM((H // 2, NPRE * PR, 6 * DH), F32),
            pltpu.SemaphoreType.DMA((4, H // 2)),
            pltpu.SemaphoreType.DMA((3 * D // 128,)),
            pltpu.SemaphoreType.DMA((5,)),
            pltpu.SemaphoreType.DMA((1,)),
        ],
        compiler_params=pltpu.CompilerParams(vmem_limit_bytes=120 * 1024 * 1024),
    )(A_x.reshape(S // SEG, SEG, D), A_mem0.reshape(M, D), wt(A_Wq), wt(A_Wk), wt(A_Wv),
      A_Wo.reshape(H * DH, D), B_wqkv, B_wo)
    return out.reshape(B, S, D)
```

```python
import functools

import jax
import jax.numpy as jnp
import numpy as np
from jax import lax
from jax.experimental import pallas as pl
from jax.experimental.pallas import tpu as pltpu

F32 = jnp.float32
BF16 = jnp.bfloat16
U32 = jnp.uint32
NEG = -1000000000.0

NPRE = 38

PR = 8
UNROLL = 2


def _bf16_const(v):
    return float(np.asarray(v, dtype=BF16).astype(np.float32))


def _dot(a, b):
    return lax.dot_general(a, b, (((1,), (0,)), ((), ())), preferred_element_type=F32)


def _dot_nt(a, b):
    return lax.dot_general(a, b, (((1,), (1,)), ((), ())), preferred_element_type=F32)


def _layernorm(x):
    m = jnp.mean(x, axis=-1, keepdims=True)
    c = x - m
    v = jnp.mean(c * c, axis=-1, keepdims=True)
    return c * lax.rsqrt(v + 1e-5)


def _pack(x):
    return pltpu.bitcast(x, U32)


def _unpack(x):
    return pltpu.bitcast(x, BF16)


def _recip(d):
    r = pl.reciprocal(d, approx=True)
    return r * (2.0 - d * r)


ORDER_PRE = (
    "k0 q0 v0 q1 s0 k1 v1 q2 s1 p0 k2 q3 v2 s2 p1 k3 v3 q4 s3 p2 k4 v4 q5 s4 p3 k5 v5 q6 s5 "
    "p4 k6 v6 q7 s6 p5 k7 v7 q8 o0 s7 p6 v8 k8 o1 B q9 s8 p7 v9 k9 o2 q10 s9 p8 k10 o3 v10 "
    "q11 s10 p9 k11 v11 o4 q12 s11 p10 k12 v12 o5 q13 s12 p11 k13 v13 o6 q14 s13 p12 v14 k14 "
    "o7 q15 s14 p13 k15 v15 o9 o8 s15 p14 o12 o11 o13 o10 p15 o14 o15 b0 b2 b1 ")
ORDER_MAIN = (
    "q0 k0 v0 q1 s0 k1 v1 q2 s1 k2 v2 v3 p0 q3 s2 k3 p1 q4 s3 k4 v4 p2 q5 k5 v5 s4 q6 p3 s5 "
    "k6 v6 p4 q7 s6 o0 k7 v7 o1 p5 q8 s7 k8 v8 p6 B o2 q9 s8 k9 v9 q10 s9 p7 o3 k10 p8 v10 "
    "q11 s10 o4 k11 p9 v11 q12 s11 o5 k12 v12 q13 p10 s12 v13 k13 o6 p11 q14 s13 k14 o7 v14 "
    "p12 q15 s14 o8 k15 v15 p13 s15 p14 o10 o9 o11 o13 o14 o12 p15 b0 o15 b1 b2 ")


def _schedule(order, n_window, n_tiles):
    names = {"q": "q", "k": "k", "v": "v", "s": "qk", "p": "pv", "o": "out", "B": "bout", "b": "bproj"}
    mm = [(names[t[0]],) + ((int(t[1:]),) if t[1:] else ()) for t in order.split()]
    bwork = ([("blog", w) for w in range(n_window)] + [("bsm",)]
             + [("bpv", j) for j in range(n_tiles)])
    every = max(1, mm.index(("bout",)) // len(bwork))
    last_out = max(i for i, op in enumerate(mm) if op[0] == "out")
    s = []
    for i, op in enumerate(mm):
        if op == ("bout",):
            s += bwork
            bwork = []
        s.append(op)
        if op[0] == "qk":
            s += [("max", op[1]), ("exp", op[1])]
        if bwork and i % every == every - 1:
            s.append(bwork.pop(0))
        if op == ("bout",):
            s += [("xcvt",), ("bln",), ("hln",)]
        if i == last_out:
            s.append(("xupd",))
    return s


def _kernel(x_hbm, mem0_ref, wqt_hbm, wkt_hbm, wvt_hbm, wo_hbm, bqkv_hbm, bwo_hbm,
            out_hbm,
            xs, w_s, wo_s, bqkv_s, bwo_s, hbuf, hbbuf, qbuf, kbuf, vbuf,
            x_st, q_st, k_st, v_st, o_st, bqkv_st, bwo_st, out_st, g_s, xp_st, hall_s, pre_s,
            wsem, bsem, msem, osem,
            *, S, D, H, DH, M, SEG, W, DIL, HB):
    NSEG = S // SEG
    NG = 2 * NSEG
    L = M + SEG
    NP = H // 2
    PW = 2 * DH
    NT = D // 128
    DB = D // HB
    NU = 3 * NT
    TAIL = 16
    OC = 256
    NOC = S // OC
    X0 = 256 // SEG
    a_scale = _bf16_const(DH ** -0.5)
    b_scale = _bf16_const(DB ** -0.5)
    assert DIL * (W - 1) <= TAIL and 128 % HB == 0 and NU <= NP - 1

    def wcopies(p):
        r = pl.ds(p * PW, PW)
        return [pltpu.make_async_copy(src.at[r, :], dst.at[r, :], wsem.at[i, p])
                for i, (src, dst) in enumerate(
                    ((wqt_hbm, q_st), (wkt_hbm, k_st), (wvt_hbm, v_st), (wo_hbm, o_st)))]

    def bcopy(u):
        r = pl.ds(pl.multiple_of((u % NT) * 128, 128), 128)
        c = pl.ds(pl.multiple_of((u // NT) * D, 128), D)
        return pltpu.make_async_copy(bqkv_hbm.at[r, c], bqkv_st.at[r, c], bsem.at[u])

    def ocopy(lo, hi):
        return pltpu.make_async_copy(out_st.at[pl.ds(lo, hi - lo), :],
                                     out_hbm.at[pl.ds(lo, hi - lo), :], osem.at[0])

    cp_x0 = pltpu.make_async_copy(x_hbm.at[0:2], x_st.at[0:2], msem.at[0])
    cp_x0b = pltpu.make_async_copy(x_hbm.at[2:X0], x_st.at[2:X0], msem.at[1])
    cp_x1 = pltpu.make_async_copy(x_hbm.at[X0:NSEG], x_st.at[X0:NSEG], msem.at[2])
    cp_xp = pltpu.make_async_copy(x_hbm.at[1:NPRE + 1, SEG - PR:SEG, :], xp_st, msem.at[3])
    cp_bo = pltpu.make_async_copy(bwo_hbm, bwo_st, msem.at[4])
    cp_q0, cp_k0, cp_v0, cp_o0 = wcopies(0)

    def rows(seg):
        return pl.ds(pl.multiple_of(seg * SEG, SEG), SEG)

    def gather_heads(t):
        n = 128 // HB
        return jnp.concatenate(
            [g_s[pl.ds(n * t + dd, HB, stride=DB), :] for dd in range(n)], axis=0)

    def perm_wqkv_piece(u):
        j, a = u // NT, u % NT
        r = pl.ds(pl.multiple_of(a * 128, 128), 128)
        for f in range(NT):
            c = pl.ds(pl.multiple_of(j * D + f * 128, 128), 128)
            g_s[f * 128:(f + 1) * 128, :] = bqkv_st[r, c].astype(F32).T
        for t in range(NT):
            c = pl.ds(pl.multiple_of(j * D + t * 128, 128), 128)
            bqkv_s[pl.ds(pl.multiple_of(a * 64, 64), 64), c] = _pack(gather_heads(t).T.astype(BF16))

    def perm_wo():
        for f in range(NT):
            c = slice(f * 128, (f + 1) * 128)
            g_s[...] = bwo_st[:, c].astype(F32)
            for t in range(NT):
                bwo_s[t * 64:(t + 1) * 64, c] = _pack(gather_heads(t).astype(BF16))

    def b_ln(seg):
        hbbuf[...] = _layernorm(xs[rows(seg), :])

    def b_proj(seg, j):
        y = _dot(hbbuf[...], _unpack(bqkv_s[:, j * D:(j + 1) * D]))
        if j == 0:
            qbuf[...] = y * b_scale
        else:
            buf = kbuf if j == 1 else vbuf
            buf[0:TAIL, :] = jnp.where(seg == 0, 0.0, buf[SEG:SEG + TAIL, :])
            buf[TAIL:, :] = y

    def b_logit(st, seg, w):
        off = TAIL - DIL * w
        s = None
        for j in range(NT):
            c = slice(j * 128, (j + 1) * 128)
            t = qbuf[:, c] * kbuf[off:off + SEG, c]
            s = t if s is None else s + t
        s = s + pltpu.roll(s, 64, 1)
        s = s + pltpu.roll(s, 32, 1)
        if w > 0:
            pos = lax.broadcasted_iota(jnp.int32, (SEG, 128), 0) + seg * SEG
            s = jnp.where(pos >= DIL * w, s, NEG)
        st.setdefault("blog", []).append(s)

    def b_softmax(st):
        logits = st["blog"]
        m = functools.reduce(jnp.maximum, logits)
        st["bexp"] = [jnp.exp(s - m) for s in logits]
        st["binv"] = _recip(functools.reduce(jnp.add, st["bexp"]))

    def b_pv(st, j):
        c = slice(j * 128, (j + 1) * 128)
        oj = None
        for w in range(W):
            off = TAIL - DIL * w
            t = st["bexp"][w] * vbuf[off:off + SEG, c]
            oj = t if oj is None else oj + t
        st.setdefault("bo", []).append(oj * st["binv"])

    def b_out(st, seg, active):
        x1 = xs[rows(seg), :]
        x2 = x1 + _dot(jnp.concatenate(st["bo"], axis=1), _unpack(bwo_s[...]))
        x2 = jnp.where(active, x2, x1)
        xs[rows(seg), :] = x2
        out_st[rows(seg), :] = x2.astype(out_st.dtype)

    def a_proj(st, p, j):
        h = st["h"][st["r0"]:, :] if j == 0 else st["h"]
        y = _dot(h, _unpack(w_s[p, :, j * PW:(j + 1) * PW]))
        if "pre" in st:
            y = jnp.concatenate([y, pre_s[p, st["pre"], j * PW:(j + 1) * PW]], axis=0)
        st["qkv"[j], p] = y

    def split_heads(t):
        lo = lax.broadcasted_iota(jnp.int32, (L, 128), 1) < (DH - 128)
        z = jnp.zeros((L, 128), F32)
        t0, t1, t2 = t[:, 0:128], t[:, 128:256], t[:, 256:384]
        top = jnp.concatenate([t0, jnp.where(lo, t1, 0.0), z], axis=1)
        bot = jnp.concatenate([z, jnp.where(lo, 0.0, t1), t2], axis=1)
        return jnp.concatenate([top, bot], axis=0).astype(BF16)

    def score_masks(r0=0):
        row = lax.broadcasted_iota(jnp.int32, (L - r0, 128), 0) + r0
        col = lax.broadcasted_iota(jnp.int32, (L - r0, 128), 1)
        lo = col < L
        key = jnp.where(lo, col, col - L)
        visible = ((row < M) | (row >= key)) & (col < 2 * L)
        fill = jnp.where(col < 2 * L, NEG, -jnp.inf)
        return lo, visible, fill

    def a_qk(st, p):
        st["s", p] = _dot_nt(st["q", p], split_heads(st["k", p]))

    def a_max(st, p):
        lo, visible, fill = score_masks(st["r0"])
        s = jnp.concatenate([st["s", p], jnp.zeros((L - st["r0"], 128 - 2 * L), F32)], axis=1)
        s = jnp.where(visible, s * a_scale, fill)
        m_lo = jnp.max(jnp.where(lo, s, -jnp.inf), axis=-1, keepdims=True)
        m_hi = jnp.max(jnp.where(lo, -jnp.inf, s), axis=-1, keepdims=True)
        st["s", p] = s
        st["m", p] = (m_lo, m_hi)

    def a_exp(st, p):
        lo = score_masks(st["r0"])[0]
        m_lo, m_hi = st["m", p]
        e = jnp.exp(st["s", p] - jnp.where(lo, m_lo, m_hi))
        d_lo = jnp.sum(jnp.where(lo, e, 0.0), axis=-1, keepdims=True)
        d_hi = jnp.sum(jnp.where(lo, 0.0, e), axis=-1, keepdims=True)
        st["e", p] = e
        st["d", p] = (d_lo, d_hi)

    def a_norm(st, p):
        lo = score_masks(st["r0"])[0]
        d_lo, d_hi = st["d", p]
        vb = jnp.concatenate([split_heads(st["v", p]), jnp.zeros((128 - 2 * L, PW), BF16)], axis=0)
        return st["e", p] * _recip(jnp.where(lo, d_lo, d_hi)), vb

    def a_pv(st, p):
        st["o", p] = _dot(*a_norm(st, p))

    def a_out(st, p):
        y = _dot(st["o", p], _unpack(wo_s[p]))
        st["acc"] = y if "acc" not in st else st["acc"] + y

    cp_x0.start()
    cp_xp.start()
    cp_q0.start()

    kbuf[...] = jnp.zeros(kbuf.shape, F32)
    vbuf[...] = jnp.zeros(vbuf.shape, F32)
    qbuf[...] = jnp.zeros(qbuf.shape, F32)
    hbbuf[...] = jnp.zeros(hbbuf.shape, F32)
    mem0 = mem0_ref[...].astype(F32)

    def load_x(lo, hi):
        for i in range(lo, hi):
            xs[i * SEG:(i + 1) * SEG, :] = x_st[i].astype(F32)

    cp_k0.start()
    cp_x0.wait()
    load_x(0, 2)
    cp_xp.wait()
    cp_v0.start()
    hall_s[0:M, :] = mem0
    hall_s[M:L, :] = _layernorm(xs[0:SEG, :])
    hall_s[L:, :] = _layernorm(xp_st[...].astype(F32).reshape(NPRE * PR, D))

    def start_pair(p):
        for cp in wcopies(p):
            cp.start()
        bcopy(p).start()

    def first_pair(p, carry, head=False):
        acc, pr_prev, vb_prev = carry
        r = pl.ds(pl.multiple_of(p * PW, PW), PW)
        st = {"r0": 0}

        def proj(j):
            y = _dot_nt(hall_s[...], (q_st, k_st, v_st)[j][r, :])
            st["qkv"[j], 0] = y[:L, :]
            pre_s[p, :, j * PW:(j + 1) * PW] = y[L:, :]

        def repack(j):
            w_s[p, :, j * PW:(j + 1) * PW] = _pack((q_st, k_st, v_st)[j][r, :].T)

        if head:
            cp_q0.wait()
            cp_o0.start()
            bcopy(0).start()
            cp_x0b.start()
            proj(0)
            cp_k0.wait()
            bcopy(0).wait()
            start_pair(1)
            proj(1)
            repack(0)
            a_qk(st, 0)
            perm_wqkv_piece(0)
            cp_v0.wait()
            cp_o0.wait()
            start_pair(2)
            proj(2)
            repack(1)
            a_max(st, 0)
            a_exp(st, 0)
            repack(2)
            wo_s[p] = _pack(o_st[r, :])
            return (acc,) + a_norm(st, 0)

        for cp in wcopies(p):
            cp.wait()

        @pl.when(p < NU)
        def _():
            bcopy(jnp.minimum(p, NU - 1)).wait()

        @pl.when(p + 2 < NP)
        def _():
            for cp in wcopies(jnp.minimum(p + 2, NP - 1)):
                cp.start()

        @pl.when(p + 2 < NU)
        def _():
            bcopy(jnp.minimum(p + 2, NU - 1)).start()

        @pl.when(p + 2 == NP)
        def _():
            cp_bo.start()
            cp_x1.start()

        rprev = pl.ds(pl.multiple_of(jnp.maximum(p - 1, 0) * PW, PW), PW)
        proj(0)
        o_prev = _dot(pr_prev, vb_prev)
        proj(1)
        acc = acc + _dot(o_prev, o_st[rprev, :])
        a_qk(st, 0)
        repack(0)
        proj(2)
        a_max(st, 0)
        perm_wqkv_piece(jnp.minimum(p, NU - 1))
        repack(1)
        a_exp(st, 0)
        repack(2)
        wo_s[p] = _pack(o_st[r, :])
        return (acc,) + a_norm(st, 0)

    carry = first_pair(0, (jnp.zeros((L, D), F32), None, None), head=True)
    acc0, pr, vb = lax.fori_loop(1, NP, first_pair, carry)
    cp_x0b.wait()
    load_x(2, X0)
    cp_bo.wait()
    acc0 = acc0 + _dot(_dot(pr, vb), o_st[(NP - 1) * PW:NP * PW, :])
    perm_wo()
    xs[0:SEG, :] = xs[0:SEG, :] + acc0[M:, :]
    hbuf[...] = _layernorm(xs[SEG:2 * SEG, :])

    GX = X0 - 1 - (X0 - 2) % UNROLL
    assert NPRE % UNROLL == 0 and (NG - 2 - NPRE) % UNROLL == 0 and X0 <= NPRE < NSEG
    assert X0 + 2 * (NPRE - GX) + 1 >= NSEG - 1
    assert NP == 16
    schedules = {True: _schedule(ORDER_PRE, W, NT), False: _schedule(ORDER_MAIN, W, NT)}

    def step(g, mem, pre=False, last=False):
        seg = g % NSEG
        seg1 = (g + NSEG - 1) % NSEG
        seg2 = jnp.maximum(g - 2, 0) % NSEG
        segn = (g + 1) % NSEG
        mem = jnp.where(seg == 0, mem0, mem)
        first_out = NSEG + OC // SEG + 2

        @pl.when((g >= first_out) & ((g - first_out) % (OC // SEG) == 0))
        def _():
            lo = pl.multiple_of((g - first_out) // (OC // SEG) * OC, OC)
            ocopy_dyn(lo).start()

        if pre:
            st = {"h": jnp.concatenate([mem, hbuf[0:SEG - PR, :]], axis=0).astype(BF16),
                  "pre": pl.ds(pl.multiple_of((g - 1) * PR, PR), PR)}
        else:
            st = {"h": jnp.concatenate([mem, hbuf[...]], axis=0)}
        r0 = st["r0"] = M if last else 0

        for op, *arg in schedules[pre]:
            if op in ("q", "k", "v"):
                a_proj(st, arg[0], "qkv".index(op))
            elif op == "qk":
                a_qk(st, arg[0])
            elif op == "max":
                a_max(st, arg[0])
            elif op == "exp":
                a_exp(st, arg[0])
            elif op == "pv":
                a_pv(st, arg[0])
            elif op == "out":
                a_out(st, arg[0])
            elif op == "blog":
                b_logit(st, seg2, arg[0])
            elif op == "bsm":
                b_softmax(st)
            elif op == "bpv":
                b_pv(st, arg[0])
            elif op == "bout":
                b_out(st, seg2, g >= 2)
            elif op == "bln":
                b_ln(seg1)
            elif op == "bproj":
                b_proj(seg1, arg[0])
            elif op == "xupd":
                xs[rows(seg), :] = xs[rows(seg), :] + st["acc"][M - r0:, :]
            elif op == "xcvt":
                if pre:
                    for u in range(2):
                        c = jnp.where(g >= GX, jnp.minimum(X0 + 2 * (g - GX) + u, NSEG - 1), X0 - 1)
                        xs[rows(c), :] = x_st[c].astype(F32)
            elif op == "hln":
                if not last:
                    hbuf[...] = _layernorm(xs[rows(segn), :])
            else:
                raise ValueError(op)
        return None if last else st["acc"][:M, :]

    def ocopy_dyn(lo):
        r = pl.ds(lo, OC)
        return pltpu.make_async_copy(out_st.at[r, :], out_hbm.at[r, :], osem.at[0])

    def body_pre(i, mem):
        @pl.when(i == GX // UNROLL)
        def _():
            cp_x1.wait()
        for u in range(UNROLL):
            mem = step(1 + i * UNROLL + u, mem, pre=True)
        return mem

    def body(i, mem):
        for u in range(UNROLL):
            mem = step(1 + NPRE + i * UNROLL + u, mem)
        return mem

    mem = lax.fori_loop(0, NPRE // UNROLL, body_pre, acc0[:M, :])
    mem = lax.fori_loop(0, (NG - 2 - NPRE) // UNROLL, body, mem)
    step(NG - 1, mem, last=True)

    last = S - 2 * SEG
    cp_last = [ocopy(S - OC, last), ocopy(last, S)]
    cp_last[0].start()
    for seg in (NSEG - 2, NSEG - 1):
        st = {}
        for w in range(W):
            b_logit(st, seg, w)
        b_softmax(st)
        for j in range(NT):
            b_pv(st, j)
        if seg == NSEG - 2:
            b_ln(NSEG - 1)
        b_out(st, seg, True)
        if seg == NSEG - 2:
            for j in range(3):
                b_proj(NSEG - 1, j)
    cp_last[1].start()
    for c in range(NOC - 1):
        ocopy(c * OC, (c + 1) * OC).wait()
    for cp in cp_last:
        cp.wait()


@functools.partial(jax.jit, static_argnames=("A_seg_len",))
def pallas_interleave_layers__memory_aug_recurrent_mem_tr__sliding_local_dilated__prompt_kernel(
    A_x, A_mem0, A_Wq, A_Wk, A_Wv, A_Wo, A_seg_len, B_x, B_wqkv, B_wo,
):
    del B_x
    B, S, D = A_x.shape
    M = A_mem0.shape[1]
    _, H, DH = A_Wq.shape
    SEG = int(A_seg_len)
    HB, W, DIL = 32, 8, 2
    assert B == 1 and S % 256 == 0 and H % 2 == 0 and 2 * DH == 384 and D % 128 == 0

    def wt(w):
        return w.transpose(1, 2, 0).reshape(H * DH, D)

    hbm = pl.BlockSpec(memory_space=pl.ANY)
    out = pl.pallas_call(
        functools.partial(_kernel, S=S, D=D, H=H, DH=DH, M=M, SEG=SEG, W=W, DIL=DIL, HB=HB),
        out_shape=jax.ShapeDtypeStruct((S, D), A_x.dtype),
        in_specs=[hbm, pl.BlockSpec(memory_space=pltpu.VMEM), hbm, hbm, hbm, hbm, hbm, hbm],
        out_specs=hbm,
        scratch_shapes=[
            pltpu.VMEM((S, D), F32),
            pltpu.VMEM((H // 2, D // 2, 6 * DH), U32),
            pltpu.VMEM((H // 2, DH, D), U32),
            pltpu.VMEM((D // 2, 3 * D), U32),
            pltpu.VMEM((D // 2, D), U32),
            pltpu.VMEM((SEG, D), F32),
            pltpu.VMEM((SEG, D), F32),
            pltpu.VMEM((SEG, D), F32),
            pltpu.VMEM((16 + SEG, D), F32),
            pltpu.VMEM((16 + SEG, D), F32),
            pltpu.VMEM((S // SEG, SEG, D), BF16),
            pltpu.VMEM((H * DH, D), BF16),
            pltpu.VMEM((H * DH, D), BF16),
            pltpu.VMEM((H * DH, D), BF16),
            pltpu.VMEM((H * DH, D), BF16),
            pltpu.VMEM((D, 3 * D), BF16),
            pltpu.VMEM((D, D), BF16),
            pltpu.VMEM((S, D), BF16),
            pltpu.VMEM((D, 128), F32),
            pltpu.VMEM((NPRE, PR, D), BF16),
            pltpu.VMEM((M + SEG + NPRE * PR, D), F32),
            pltpu.VMEM((H // 2, NPRE * PR, 6 * DH), F32),
            pltpu.SemaphoreType.DMA((4, H // 2)),
            pltpu.SemaphoreType.DMA((3 * D // 128,)),
            pltpu.SemaphoreType.DMA((5,)),
            pltpu.SemaphoreType.DMA((1,)),
        ],
        compiler_params=pltpu.CompilerParams(vmem_limit_bytes=120 * 1024 * 1024),
    )(A_x.reshape(S // SEG, SEG, D), A_mem0.reshape(M, D), wt(A_Wq), wt(A_Wk), wt(A_Wv),
      A_Wo.reshape(H * DH, D), B_wqkv, B_wo)
    return out.reshape(B, S, D)
```

```python
import functools

import jax
import jax.numpy as jnp
import numpy as np
from jax import lax
from jax.experimental import pallas as pl
from jax.experimental.pallas import tpu as pltpu

F32 = jnp.float32
BF16 = jnp.bfloat16
U32 = jnp.uint32
NEG = -1000000000.0

NPRE = 38

PR = 8
UNROLL = 2


def _bf16_const(v):
    return float(np.asarray(v, dtype=BF16).astype(np.float32))


def _dot(a, b):
    return lax.dot_general(a, b, (((1,), (0,)), ((), ())), preferred_element_type=F32)


def _dot_nt(a, b):
    return lax.dot_general(a, b, (((1,), (1,)), ((), ())), preferred_element_type=F32)


def _layernorm(x):
    m = jnp.mean(x, axis=-1, keepdims=True)
    c = x - m
    v = jnp.mean(c * c, axis=-1, keepdims=True)
    return c * lax.rsqrt(v + 1e-5)


def _pack(x):
    return pltpu.bitcast(x, U32)


def _unpack(x):
    return pltpu.bitcast(x, BF16)


def _recip(d):
    r = pl.reciprocal(d, approx=True)
    return r * (2.0 - d * r)


ORDER_PRE = (
    "k0 q0 v0 q1 s0 k1 v1 q2 s1 p0 k2 q3 v2 s2 p1 k3 v3 q4 s3 p2 k4 v4 q5 s4 p3 k5 v5 q6 s5 "
    "p4 k6 v6 q7 s6 p5 k7 v7 q8 o0 s7 p6 v8 k8 o1 B q9 s8 p7 v9 k9 o2 q10 s9 p8 k10 o3 v10 "
    "q11 s10 p9 k11 v11 o4 q12 s11 p10 k12 v12 o5 q13 s12 p11 k13 v13 o6 q14 s13 p12 v14 k14 "
    "o7 q15 s14 p13 k15 v15 o9 o8 s15 p14 o12 o11 o13 o10 p15 o14 o15 b0 b2 b1 ")
ORDER_MAIN = (
    "q0 k0 v0 q1 s0 k1 v1 q2 s1 k2 v2 v3 p0 q3 s2 k3 p1 q4 s3 k4 v4 p2 q5 k5 v5 s4 q6 p3 s5 "
    "k6 v6 p4 q7 s6 o0 k7 v7 o1 p5 q8 s7 k8 v8 p6 B o2 q9 s8 k9 v9 q10 s9 p7 o3 k10 p8 v10 "
    "q11 s10 o4 k11 p9 v11 q12 s11 o5 k12 v12 q13 p10 s12 v13 k13 o6 p11 q14 s13 k14 o7 v14 "
    "p12 q15 s14 o8 k15 v15 p13 s15 p14 o10 o9 o11 o13 o14 o12 p15 b0 o15 b1 b2 ")


def _schedule(order, n_window, n_tiles):
    names = {"q": "q", "k": "k", "v": "v", "s": "qk", "p": "pv", "o": "out", "B": "bout", "b": "bproj"}
    mm = [(names[t[0]],) + ((int(t[1:]),) if t[1:] else ()) for t in order.split()]
    bwork = ([("blog", w) for w in range(n_window)] + [("bsm",)]
             + [("bpv", j) for j in range(n_tiles)])
    every = max(1, mm.index(("bout",)) // len(bwork))
    last_out = max(i for i, op in enumerate(mm) if op[0] == "out")
    s = []
    for i, op in enumerate(mm):
        if op == ("bout",):
            s += bwork
            bwork = []
        s.append(op)
        if op[0] == "qk":
            s += [("max", op[1]), ("exp", op[1])]
        if bwork and i % every == every - 1:
            s.append(bwork.pop(0))
        if op == ("bout",):
            s += [("xcvt",), ("bln",), ("hln",)]
        if i == last_out:
            s.append(("xupd",))
    return s


def _kernel(x_hbm, mem0_ref, wqt_hbm, wkt_hbm, wvt_hbm, wo_hbm, bqkv_hbm, bwo_hbm,
            out_hbm,
            xs, w_s, wo_s, bqkv_s, bwo_s, hbuf, hbbuf, qbuf, kbuf, vbuf,
            x_st, q_st, k_st, v_st, o_st, bqkv_st, bwo_st, out_st, g_s, xp_st, hall_s, pre_s,
            wsem, bsem, msem, osem,
            *, S, D, H, DH, M, SEG, W, DIL, HB):
    NSEG = S // SEG
    NG = 2 * NSEG
    L = M + SEG
    NP = H // 2
    PW = 2 * DH
    NT = D // 128
    DB = D // HB
    NU = 3 * NT
    TAIL = 16
    OC = 256
    NOC = S // OC
    X0 = 256 // SEG
    a_scale = _bf16_const(DH ** -0.5)
    b_scale = _bf16_const(DB ** -0.5)
    assert DIL * (W - 1) <= TAIL and 128 % HB == 0 and NU <= NP - 1

    def wcopies(p):
        r = pl.ds(p * PW, PW)
        return [pltpu.make_async_copy(src.at[r, :], dst.at[r, :], wsem.at[i, p % 2])
                for i, (src, dst) in enumerate(
                    ((wqt_hbm, q_st), (wkt_hbm, k_st), (wvt_hbm, v_st), (wo_hbm, o_st)))]

    def bcopy(u):
        r = pl.ds(pl.multiple_of((u % NT) * 128, 128), 128)
        c = pl.ds(pl.multiple_of((u // NT) * D, 128), D)
        return pltpu.make_async_copy(bqkv_hbm.at[r, c], bqkv_st.at[r, c], bsem.at[u % 2])

    def ocopy(lo, hi):
        return pltpu.make_async_copy(out_st.at[pl.ds(lo, hi - lo), :],
                                     out_hbm.at[pl.ds(lo, hi - lo), :], osem.at[0])

    cp_x0 = pltpu.make_async_copy(x_hbm.at[0:2], x_st.at[0:2], msem.at[0])
    cp_x0b = pltpu.make_async_copy(x_hbm.at[2:X0], x_st.at[2:X0], msem.at[1])
    cp_x1 = pltpu.make_async_copy(x_hbm.at[X0:NSEG], x_st.at[X0:NSEG], msem.at[2])
    cp_xp = pltpu.make_async_copy(x_hbm.at[1:NPRE + 1, SEG - PR:SEG, :], xp_st, msem.at[3])
    cp_bo = pltpu.make_async_copy(bwo_hbm, bwo_st, msem.at[4])
    cp_q0, cp_k0, cp_v0, cp_o0 = wcopies(0)

    def rows(seg):
        return pl.ds(pl.multiple_of(seg * SEG, SEG), SEG)

    def gather_heads(t):
        n = 128 // HB
        return jnp.concatenate(
            [g_s[pl.ds(n * t + dd, HB, stride=DB), :] for dd in range(n)], axis=0)

    def perm_wqkv_piece(u):
        j, a = u // NT, u % NT
        r = pl.ds(pl.multiple_of(a * 128, 128), 128)
        for f in range(NT):
            c = pl.ds(pl.multiple_of(j * D + f * 128, 128), 128)
            g_s[f * 128:(f + 1) * 128, :] = bqkv_st[r, c].astype(F32).T
        for t in range(NT):
            c = pl.ds(pl.multiple_of(j * D + t * 128, 128), 128)
            bqkv_s[pl.ds(pl.multiple_of(a * 64, 64), 64), c] = _pack(gather_heads(t).T.astype(BF16))

    def perm_wo():
        for f in range(NT):
            c = slice(f * 128, (f + 1) * 128)
            g_s[...] = bwo_st[:, c].astype(F32)
            for t in range(NT):
                bwo_s[t * 64:(t + 1) * 64, c] = _pack(gather_heads(t).astype(BF16))

    def b_ln(seg):
        hbbuf[...] = _layernorm(xs[rows(seg), :])

    def b_proj(seg, j):
        y = _dot(hbbuf[...], _unpack(bqkv_s[:, j * D:(j + 1) * D]))
        if j == 0:
            qbuf[...] = y * b_scale
        else:
            buf = kbuf if j == 1 else vbuf
            buf[0:TAIL, :] = jnp.where(seg == 0, 0.0, buf[SEG:SEG + TAIL, :])
            buf[TAIL:, :] = y

    def b_logit(st, seg, w):
        off = TAIL - DIL * w
        s = None
        for j in range(NT):
            c = slice(j * 128, (j + 1) * 128)
            t = qbuf[:, c] * kbuf[off:off + SEG, c]
            s = t if s is None else s + t
        s = s + pltpu.roll(s, 64, 1)
        s = s + pltpu.roll(s, 32, 1)
        if w > 0:
            pos = lax.broadcasted_iota(jnp.int32, (SEG, 128), 0) + seg * SEG
            s = jnp.where(pos >= DIL * w, s, NEG)
        st.setdefault("blog", []).append(s)

    def b_softmax(st):
        logits = st["blog"]
        m = functools.reduce(jnp.maximum, logits)
        st["bexp"] = [jnp.exp(s - m) for s in logits]
        st["binv"] = _recip(functools.reduce(jnp.add, st["bexp"]))

    def b_pv(st, j):
        c = slice(j * 128, (j + 1) * 128)
        oj = None
        for w in range(W):
            off = TAIL - DIL * w
            t = st["bexp"][w] * vbuf[off:off + SEG, c]
            oj = t if oj is None else oj + t
        st.setdefault("bo", []).append(oj * st["binv"])

    def b_out(st, seg, active):
        x1 = xs[rows(seg), :]
        x2 = x1 + _dot(jnp.concatenate(st["bo"], axis=1), _unpack(bwo_s[...]))
        x2 = jnp.where(active, x2, x1)
        xs[rows(seg), :] = x2
        out_st[rows(seg), :] = x2.astype(out_st.dtype)

    def a_proj(st, p, j):
        h = st["h"][st["r0"]:, :] if j == 0 else st["h"]
        y = _dot(h, _unpack(w_s[p, :, j * PW:(j + 1) * PW]))
        if "pre" in st:
            y = jnp.concatenate([y, pre_s[p, st["pre"], j * PW:(j + 1) * PW]], axis=0)
        st["qkv"[j], p] = y

    def split_heads(t):
        lo = lax.broadcasted_iota(jnp.int32, (L, 128), 1) < (DH - 128)
        z = jnp.zeros((L, 128), F32)
        t0, t1, t2 = t[:, 0:128], t[:, 128:256], t[:, 256:384]
        top = jnp.concatenate([t0, jnp.where(lo, t1, 0.0), z], axis=1)
        bot = jnp.concatenate([z, jnp.where(lo, 0.0, t1), t2], axis=1)
        return jnp.concatenate([top, bot], axis=0).astype(BF16)

    def score_masks(r0=0):
        row = lax.broadcasted_iota(jnp.int32, (L - r0, 128), 0) + r0
        col = lax.broadcasted_iota(jnp.int32, (L - r0, 128), 1)
        lo = col < L
        key = jnp.where(lo, col, col - L)
        visible = ((row < M) | (row >= key)) & (col < 2 * L)
        fill = jnp.where(col < 2 * L, NEG, -jnp.inf)
        return lo, visible, fill

    def a_qk(st, p):
        st["s", p] = _dot_nt(st["q", p], split_heads(st["k", p]))

    def a_max(st, p):
        lo, visible, fill = score_masks(st["r0"])
        s = jnp.concatenate([st["s", p], jnp.zeros((L - st["r0"], 128 - 2 * L), F32)], axis=1)
        s = jnp.where(visible, s * a_scale, fill)
        m_lo = jnp.max(jnp.where(lo, s, -jnp.inf), axis=-1, keepdims=True)
        m_hi = jnp.max(jnp.where(lo, -jnp.inf, s), axis=-1, keepdims=True)
        st["s", p] = s
        st["m", p] = (m_lo, m_hi)

    def a_exp(st, p):
        lo = score_masks(st["r0"])[0]
        m_lo, m_hi = st["m", p]
        e = jnp.exp(st["s", p] - jnp.where(lo, m_lo, m_hi))
        d_lo = jnp.sum(jnp.where(lo, e, 0.0), axis=-1, keepdims=True)
        d_hi = jnp.sum(jnp.where(lo, 0.0, e), axis=-1, keepdims=True)
        st["e", p] = e
        st["d", p] = (d_lo, d_hi)

    def a_norm(st, p):
        lo = score_masks(st["r0"])[0]
        d_lo, d_hi = st["d", p]
        vb = jnp.concatenate([split_heads(st["v", p]), jnp.zeros((128 - 2 * L, PW), BF16)], axis=0)
        return st["e", p] * _recip(jnp.where(lo, d_lo, d_hi)), vb

    def a_pv(st, p):
        st["o", p] = _dot(*a_norm(st, p))

    def a_out(st, p):
        y = _dot(st["o", p], _unpack(wo_s[p]))
        st["acc"] = y if "acc" not in st else st["acc"] + y

    cp_x0.start()
    cp_xp.start()
    cp_q0.start()

    kbuf[...] = jnp.zeros(kbuf.shape, F32)
    vbuf[...] = jnp.zeros(vbuf.shape, F32)
    qbuf[...] = jnp.zeros(qbuf.shape, F32)
    hbbuf[...] = jnp.zeros(hbbuf.shape, F32)
    mem0 = mem0_ref[...].astype(F32)

    def load_x(lo, hi):
        for i in range(lo, hi):
            xs[i * SEG:(i + 1) * SEG, :] = x_st[i].astype(F32)

    cp_k0.start()
    cp_x0.wait()
    load_x(0, 2)
    cp_xp.wait()
    cp_v0.start()
    hall_s[0:M, :] = mem0
    hall_s[M:L, :] = _layernorm(xs[0:SEG, :])
    hall_s[L:, :] = _layernorm(xp_st[...].astype(F32).reshape(NPRE * PR, D))

    def start_pair(p):
        for cp in wcopies(p):
            cp.start()
        bcopy(p).start()

    def first_pair(p, carry, head=False):
        acc, pr_prev, vb_prev = carry
        r = pl.ds(pl.multiple_of(p * PW, PW), PW)
        st = {"r0": 0}

        def proj(j):
            y = _dot_nt(hall_s[...], (q_st, k_st, v_st)[j][r, :])
            st["qkv"[j], 0] = y[:L, :]
            pre_s[p, :, j * PW:(j + 1) * PW] = y[L:, :]

        def repack(j):
            w_s[p, :, j * PW:(j + 1) * PW] = _pack((q_st, k_st, v_st)[j][r, :].T)

        if head:
            cp_q0.wait()
            cp_o0.start()
            bcopy(0).start()
            cp_x0b.start()
            proj(0)
            cp_k0.wait()
            bcopy(0).wait()
            start_pair(1)
            proj(1)
            repack(0)
            a_qk(st, 0)
            perm_wqkv_piece(0)
            cp_v0.wait()
            cp_o0.wait()
            start_pair(2)
            proj(2)
            repack(1)
            a_max(st, 0)
            a_exp(st, 0)
            repack(2)
            wo_s[p] = _pack(o_st[r, :])
            return (acc,) + a_norm(st, 0)

        for cp in wcopies(p):
            cp.wait()

        @pl.when(p < NU)
        def _():
            bcopy(jnp.minimum(p, NU - 1)).wait()

        @pl.when(p + 2 < NP)
        def _():
            for cp in wcopies(jnp.minimum(p + 2, NP - 1)):
                cp.start()

        @pl.when(p + 2 < NU)
        def _():
            bcopy(jnp.minimum(p + 2, NU - 1)).start()

        @pl.when(p + 2 == NP)
        def _():
            cp_bo.start()
            cp_x1.start()

        rprev = pl.ds(pl.multiple_of(jnp.maximum(p - 1, 0) * PW, PW), PW)
        proj(0)
        o_prev = _dot(pr_prev, vb_prev)
        proj(1)
        acc = acc + _dot(o_prev, o_st[rprev, :])
        a_qk(st, 0)
        repack(0)
        proj(2)
        a_max(st, 0)
        perm_wqkv_piece(jnp.minimum(p, NU - 1))
        repack(1)
        a_exp(st, 0)
        repack(2)
        wo_s[p] = _pack(o_st[r, :])
        return (acc,) + a_norm(st, 0)

    carry = first_pair(0, (jnp.zeros((L, D), F32), None, None), head=True)
    acc0, pr, vb = lax.fori_loop(1, NP, first_pair, carry)
    cp_x0b.wait()
    load_x(2, X0)
    cp_bo.wait()
    acc0 = acc0 + _dot(_dot(pr, vb), o_st[(NP - 1) * PW:NP * PW, :])
    perm_wo()
    xs[0:SEG, :] = xs[0:SEG, :] + acc0[M:, :]
    hbuf[...] = _layernorm(xs[SEG:2 * SEG, :])

    GX = X0 - 1 - (X0 - 2) % UNROLL
    assert NPRE % UNROLL == 0 and (NG - 2 - NPRE) % UNROLL == 0 and X0 <= NPRE < NSEG
    assert X0 + 2 * (NPRE - GX) + 1 >= NSEG - 1
    assert NP == 16
    schedules = {True: _schedule(ORDER_PRE, W, NT), False: _schedule(ORDER_MAIN, W, NT)}

    def step(g, mem, pre=False, last=False):
        seg = g % NSEG
        seg1 = (g + NSEG - 1) % NSEG
        seg2 = jnp.maximum(g - 2, 0) % NSEG
        segn = (g + 1) % NSEG
        mem = jnp.where(seg == 0, mem0, mem)
        first_out = NSEG + OC // SEG + 2

        @pl.when((g >= first_out) & ((g - first_out) % (OC // SEG) == 0))
        def _():
            lo = pl.multiple_of((g - first_out) // (OC // SEG) * OC, OC)
            ocopy_dyn(lo).start()

        if pre:
            st = {"h": jnp.concatenate([mem, hbuf[0:SEG - PR, :]], axis=0).astype(BF16),
                  "pre": pl.ds(pl.multiple_of((g - 1) * PR, PR), PR)}
        else:
            st = {"h": jnp.concatenate([mem, hbuf[...]], axis=0)}
        r0 = st["r0"] = M if last else 0

        for op, *arg in schedules[pre]:
            if op in ("q", "k", "v"):
                a_proj(st, arg[0], "qkv".index(op))
            elif op == "qk":
                a_qk(st, arg[0])
            elif op == "max":
                a_max(st, arg[0])
            elif op == "exp":
                a_exp(st, arg[0])
            elif op == "pv":
                a_pv(st, arg[0])
            elif op == "out":
                a_out(st, arg[0])
            elif op == "blog":
                b_logit(st, seg2, arg[0])
            elif op == "bsm":
                b_softmax(st)
            elif op == "bpv":
                b_pv(st, arg[0])
            elif op == "bout":
                b_out(st, seg2, g >= 2)
            elif op == "bln":
                b_ln(seg1)
            elif op == "bproj":
                b_proj(seg1, arg[0])
            elif op == "xupd":
                xs[rows(seg), :] = xs[rows(seg), :] + st["acc"][M - r0:, :]
            elif op == "xcvt":
                if pre:
                    for u in range(2):
                        c = jnp.where(g >= GX, jnp.minimum(X0 + 2 * (g - GX) + u, NSEG - 1), X0 - 1)
                        xs[rows(c), :] = x_st[c].astype(F32)
            elif op == "hln":
                if not last:
                    hbuf[...] = _layernorm(xs[rows(segn), :])
            else:
                raise ValueError(op)
        return None if last else st["acc"][:M, :]

    def ocopy_dyn(lo):
        r = pl.ds(lo, OC)
        return pltpu.make_async_copy(out_st.at[r, :], out_hbm.at[r, :], osem.at[0])

    def body_pre(i, mem):
        @pl.when(i == GX // UNROLL)
        def _():
            cp_x1.wait()
        for u in range(UNROLL):
            mem = step(1 + i * UNROLL + u, mem, pre=True)
        return mem

    def body(i, mem):
        for u in range(UNROLL):
            mem = step(1 + NPRE + i * UNROLL + u, mem)
        return mem

    mem = lax.fori_loop(0, NPRE // UNROLL, body_pre, acc0[:M, :])
    mem = lax.fori_loop(0, (NG - 2 - NPRE) // UNROLL, body, mem)
    step(NG - 1, mem, last=True)

    last = S - 2 * SEG
    cp_last = [ocopy(S - OC, last), ocopy(last, S)]
    cp_last[0].start()
    for seg in (NSEG - 2, NSEG - 1):
        st = {}
        for w in range(W):
            b_logit(st, seg, w)
        b_softmax(st)
        for j in range(NT):
            b_pv(st, j)
        if seg == NSEG - 2:
            b_ln(NSEG - 1)
        b_out(st, seg, True)
        if seg == NSEG - 2:
            for j in range(3):
                b_proj(NSEG - 1, j)
    cp_last[1].start()
    for c in range(NOC - 1):
        ocopy(c * OC, (c + 1) * OC).wait()
    for cp in cp_last:
        cp.wait()


@functools.partial(jax.jit, static_argnames=("A_seg_len",))
def pallas_interleave_layers__memory_aug_recurrent_mem_tr__sliding_local_dilated__prompt_kernel(
    A_x, A_mem0, A_Wq, A_Wk, A_Wv, A_Wo, A_seg_len, B_x, B_wqkv, B_wo,
):
    del B_x
    B, S, D = A_x.shape
    M = A_mem0.shape[1]
    _, H, DH = A_Wq.shape
    SEG = int(A_seg_len)
    HB, W, DIL = 32, 8, 2
    assert B == 1 and S % 256 == 0 and H % 2 == 0 and 2 * DH == 384 and D % 128 == 0

    def wt(w):
        return w.transpose(1, 2, 0).reshape(H * DH, D)

    hbm = pl.BlockSpec(memory_space=pl.ANY)
    out = pl.pallas_call(
        functools.partial(_kernel, S=S, D=D, H=H, DH=DH, M=M, SEG=SEG, W=W, DIL=DIL, HB=HB),
        out_shape=jax.ShapeDtypeStruct((S, D), A_x.dtype),
        in_specs=[hbm, pl.BlockSpec(memory_space=pltpu.VMEM), hbm, hbm, hbm, hbm, hbm, hbm],
        out_specs=hbm,
        scratch_shapes=[
            pltpu.VMEM((S, D), F32),
            pltpu.VMEM((H // 2, D // 2, 6 * DH), U32),
            pltpu.VMEM((H // 2, DH, D), U32),
            pltpu.VMEM((D // 2, 3 * D), U32),
            pltpu.VMEM((D // 2, D), U32),
            pltpu.VMEM((SEG, D), F32),
            pltpu.VMEM((SEG, D), F32),
            pltpu.VMEM((SEG, D), F32),
            pltpu.VMEM((16 + SEG, D), F32),
            pltpu.VMEM((16 + SEG, D), F32),
            pltpu.VMEM((S // SEG, SEG, D), BF16),
            pltpu.VMEM((H * DH, D), BF16),
            pltpu.VMEM((H * DH, D), BF16),
            pltpu.VMEM((H * DH, D), BF16),
            pltpu.VMEM((H * DH, D), BF16),
            pltpu.VMEM((D, 3 * D), BF16),
            pltpu.VMEM((D, D), BF16),
            pltpu.VMEM((S, D), BF16),
            pltpu.VMEM((D, 128), F32),
            pltpu.VMEM((NPRE, PR, D), BF16),
            pltpu.VMEM((M + SEG + NPRE * PR, D), F32),
            pltpu.VMEM((H // 2, NPRE * PR, 6 * DH), F32),
            pltpu.SemaphoreType.DMA((4, 2)),
            pltpu.SemaphoreType.DMA((2,)),
            pltpu.SemaphoreType.DMA((5,)),
            pltpu.SemaphoreType.DMA((1,)),
        ],
        compiler_params=pltpu.CompilerParams(vmem_limit_bytes=120 * 1024 * 1024),
    )(A_x.reshape(S // SEG, SEG, D), A_mem0.reshape(M, D), wt(A_Wq), wt(A_Wk), wt(A_Wv),
      A_Wo.reshape(H * DH, D), B_wqkv, B_wo)
    return out.reshape(B, S, D)
```
